```python
import jax
import jax.numpy as jnp

def _softmax(x, axis=-1):
    return jax.nn.softmax(x, axis=axis)

def _gelu(x):
    return jax.nn.gelu(x, approximate=True)

def _silu(x):
    return jax.nn.silu(x)

def _sigmoid(x):
    return jax.nn.sigmoid(x)

def _layernorm(x, axis=-1, eps=1e-05):
    m = jnp.mean(x, axis=axis, keepdims=True)
    v = jnp.var(x, axis=axis, keepdims=True)
    return (x - m) / jnp.sqrt(v + eps)

def _scatter_add(tgt, idx, src, axis=0):
    return tgt.at[idx].add(src)

def _segment_sum(src, seg, n):
    return jax.ops.segment_sum(src, seg, n)

class _Rng:

    def __init__(self, key):
        self._k = key

    def _next(self):
        self._k, sub = jax.random.split(self._k)
        return sub

    def normal(self, shape):
        return jax.random.normal(self._next(), shape, dtype=jnp.bfloat16)

    def randint(self, lo, hi, shape):
        return jax.random.randint(self._next(), shape, lo, hi, dtype=jnp.int32)

    def uniform(self, shape, lo=0.0, hi=1.0):
        return jax.random.uniform(self._next(), shape, jnp.bfloat16, lo, hi)

    def permutation(self, n):
        return jax.random.permutation(self._next(), n)
kernel_name = 'concat_heads__ssm_conv_s4__memory_aug_recurrent_mem_tr__prompt'

def setup_inputs():
    _rng = _Rng(jax.random.key(int.from_bytes(__import__("os").urandom(4), "little")))
    _w = lambda a: (lambda t: t.astype(jnp.bfloat16) if jnp.issubdtype(t.dtype, jnp.floating) else t)(jnp.asarray(a))

    def _A_setup():
        B, L, D, N = (1, 2048, 640, 128)
        A_re = -jnp.exp((lambda *s: _rng.normal(s) * 0.05)(D, N))
        A_im = jnp.pi * (lambda *s: _rng.normal(s) * 0.05)(D, N)
        B_re = (lambda *s: _rng.normal(s) * 0.05)(D, N)
        B_im = (lambda *s: _rng.normal(s) * 0.05)(D, N)
        C_re = (lambda *s: _rng.normal(s) * 0.05)(D, N)
        C_im = (lambda *s: _rng.normal(s) * 0.05)(D, N)
        log_dt = (lambda *s: _rng.normal(s) * 0.05)(D) * 0.5 - 4.0
        Dskip = (lambda *s: _rng.normal(s) * 0.05)(D)
        return {'u': _w((lambda *s: _rng.normal(s) * 0.05)(B, L, D)), 'A_re': _w(A_re), 'A_im': _w(A_im), 'B_re': _w(B_re), 'B_im': _w(B_im), 'C_re': _w(C_re), 'C_im': _w(C_im), 'log_dt': _w(log_dt), 'Dskip': _w(Dskip)}
    _A_in = _A_setup()

    def _B_setup():
        B, S, Dm = (1, 2048, 640)
        H, Dh = (32, 128)
        M, seg = (8, 32)
        seg = min(seg, S)
        S = S // seg * seg
        return {'x': _w((lambda *s: _rng.normal(s) * 0.05)(B, S, Dm)), 'mem0': _w((lambda *s: _rng.normal(s) * 0.05)(B, M, Dm)), 'Wq': _w((lambda *s: _rng.normal(s) * 0.05)(Dm, H, Dh) * Dm ** (-0.5)), 'Wk': _w((lambda *s: _rng.normal(s) * 0.05)(Dm, H, Dh) * Dm ** (-0.5)), 'Wv': _w((lambda *s: _rng.normal(s) * 0.05)(Dm, H, Dh) * Dm ** (-0.5)), 'Wo': _w((lambda *s: _rng.normal(s) * 0.05)(H, Dh, Dm) * (H * Dh) ** (-0.5)), 'seg_len': seg}
    _B_in = _B_setup()
    return {'A_u': _A_in['u'], 'A_A_re': _A_in['A_re'], 'A_A_im': _A_in['A_im'], 'A_B_re': _A_in['B_re'], 'A_B_im': _A_in['B_im'], 'A_C_re': _A_in['C_re'], 'A_C_im': _A_in['C_im'], 'A_log_dt': _A_in['log_dt'], 'A_Dskip': _A_in['Dskip'], 'B_x': _B_in['x'], 'B_mem0': _B_in['mem0'], 'B_Wq': _B_in['Wq'], 'B_Wk': _B_in['Wk'], 'B_Wv': _B_in['Wv'], 'B_Wo': _B_in['Wo'], 'B_seg_len': _B_in['seg_len']}

def reference(A_u, A_A_re, A_A_im, A_B_re, A_B_im, A_C_re, A_C_im, A_log_dt, A_Dskip, B_x, B_mem0, B_Wq, B_Wk, B_Wv, B_Wo, B_seg_len):

    def _A_ref(u, A_re, A_im, B_re, B_im, C_re, C_im, log_dt, Dskip):
        Bsz, L, D = u.shape
        dt = jnp.exp(log_dt)[:, None]
        A = A_re + 1j * A_im
        Bc = B_re + 1j * B_im
        Cc = C_re + 1j * C_im
        logdA = dt * A
        dB = dt * Bc
        l = (lambda x, dt: x.astype(dt))(jnp.arange(L), A_re.dtype)
        P = jnp.exp(logdA[:, :, None] * l[None, None, :])
        K = jnp.einsum('dn,dnl,dn->dl', Cc, P, dB).real
        L2 = 2 * L
        Kp = jnp.pad(K, ((0, 0), (0, L)))
        up = (lambda x, *d: x.transpose(*d))(u, 0, 2, 1)
        up = jnp.pad(up, ((0, 0), (0, 0), (0, L)))
        Kf = (lambda x, axes=(-2, -1): jnp.fft.rfft2(x.astype(jnp.float32), axes=axes))(Kp[:, None, :], axes=(-2, -1))
        Uf = (lambda x, axes=(-2, -1): jnp.fft.rfft2(x.astype(jnp.float32), axes=axes))(up[:, :, None, :], axes=(-2, -1))
        Yf = Uf * Kf[None, :, :, :]
        y = (lambda x, s, axes=(-2, -1): jnp.fft.irfft2(x, s=s, axes=axes).astype(jnp.bfloat16))(Yf, (1, L2), axes=(-2, -1))[:, :, 0, :L]
        y = (lambda x, *d: x.transpose(*d))(y, 0, 2, 1) + u * Dskip[None, None, :]
        return y

    def _B_ref(x, mem0, Wq, Wk, Wv, Wo, seg_len):
        B, S, Dm = x.shape
        H, Dh = (Wq.shape[1], Wq.shape[2])
        M = mem0.shape[1]
        scale = Dh ** (-0.5)
        n_seg = S // seg_len
        L = M + seg_len
        idx = jnp.arange(L)
        mask = (idx[:, None] < M) | (idx[:, None] >= idx[None, :])
        mem = mem0
        outs = []
        for s in range(n_seg):
            xs = x[:, s * seg_len:(s + 1) * seg_len, :].copy()
            h = jnp.concatenate([mem, xs], axis=1)
            q = jnp.einsum('btd,dhe->bhte', h, Wq)
            k = jnp.einsum('btd,dhe->bhte', h, Wk)
            v = jnp.einsum('btd,dhe->bhte', h, Wv)
            scores = jnp.einsum('bhqe,bhke->bhqk', q, k) * scale
            scores = jnp.where(mask[None, None], scores, -1000000000.0)
            p = _softmax(scores, axis=-1)
            o = jnp.einsum('bhqk,bhke->bhqe', p, v)
            o = jnp.einsum('bhte,hed->btd', o, Wo)
            mem = o[:, :M, :].copy()
            outs.append(o[:, M:, :])
        return jnp.concatenate(outs, axis=1)
    a = _A_ref(A_u, A_A_re, A_A_im, A_B_re, A_B_im, A_C_re, A_C_im, A_log_dt, A_Dskip)
    b = _B_ref(B_x, B_mem0, B_Wq, B_Wk, B_Wv, B_Wo, B_seg_len)
    return jnp.concatenate([a, b], axis=-1)
```

```python
import functools

import jax
import jax.numpy as jnp
from jax import lax
import jax.experimental.pallas as pl
import jax.experimental.pallas.tpu as pltpu

F32 = jnp.float32
BF16 = jnp.bfloat16
U32 = jnp.uint32
I32 = jnp.int32

LANES = 128
T = 64
NCH = 32
CP = NCH + 1
GP = 8
RING = 4
SKEW = (2, 4, 6, 8)


def _mm(a, b):
    return lax.dot_general(a, b, (((1,), (0,)), ((), ())), preferred_element_type=F32)


def _mm_nt(a, b):
    return lax.dot_general(a, b, (((1,), (1,)), ((), ())), preferred_element_type=F32)


def _cmul(ar, ai, br, bi):
    return ar * br - ai * bi, ar * bi + ai * br


def _iota(shape, dim):
    return lax.broadcasted_iota(I32, shape, dim)


def _kernel(u_hbm, are_ref, aim_ref, bre_ref, bim_ref, cre_ref, cim_ref, ldt_ref, dsk_ref,
            x_hbm, mem0_ref, wq_hbm, wk_hbm, wv_hbm, wo_hbm, out_hbm,
            u_v, x_v, raw_v, wqkv_v, wo_v, oa_v, ob_v, obuf,
            pw_re, pw_im, par, ut, y2, vbuf, sbuf, zbuf, ybuf, kbuf, tmask, tidx,
            sems, *, seq, dm, heads, dh, nmem, seg):
    nblk = dm // LANES
    ngrp = dm // (2 * GP)
    pp = dm + 1
    rows = nmem + seg

    cp_u = pltpu.make_async_copy(u_hbm, u_v, sems.at[0])
    cp_w = [pltpu.make_async_copy(w, raw_v.at[i], sems.at[1 + i])
            for i, w in enumerate((wq_hbm, wk_hbm, wv_hbm))]
    cp_x = pltpu.make_async_copy(x_hbm, x_v, sems.at[4])
    cp_wo = pltpu.make_async_copy(wo_hbm, wo_v, sems.at[5])
    cp_oa = pltpu.make_async_copy(oa_v, out_hbm.at[:, pl.ds(0, dm)], sems.at[6])
    cp_u.start()
    for c in cp_w:
        c.start()
    cp_x.start()
    cp_wo.start()

    dt_row = jnp.exp(ldt_ref[...].astype(F32)).astype(BF16).astype(F32).reshape(1, dm)
    for b in range(nblk):
        r0 = b * LANES
        sl = pl.ds(r0, LANES)
        dt = jnp.broadcast_to(dt_row[:, r0:r0 + LANES], (LANES, LANES)).T
        ar = dt * are_ref[sl, :].astype(F32)
        ai = dt * aim_ref[sl, :].astype(F32)
        mag = jnp.exp(ar)
        e1 = (mag * jnp.cos(ai), mag * jnp.sin(ai))
        w = _cmul(cre_ref[sl, :].astype(F32), cim_ref[sl, :].astype(F32),
                  dt * bre_ref[sl, :].astype(F32), dt * bim_ref[sl, :].astype(F32))
        g = _cmul(*w, *e1)
        e2 = _cmul(*e1, *e1)
        e3 = _cmul(*e2, *e1)
        e4 = _cmul(*e2, *e2)
        low = [(jnp.ones_like(ar), jnp.zeros_like(ar)), e1, e2, e3, e4,
               _cmul(*e4, *e1), _cmul(*e4, *e2), _cmul(*e4, *e3)]
        for k, (pr, pi) in enumerate(low):
            pw_re[pl.ds(k * pp + r0, LANES), :] = pr
            pw_im[pl.ds(k * pp + r0, LANES), :] = pi
        e8 = _cmul(*e4, *e4)
        e16 = _cmul(*e8, *e8)
        e32 = _cmul(*e16, *e16)
        e64 = _cmul(*e32, *e32)
        for k, val in enumerate((*e8, *e16, *e32, *e64, *g, w[0], -w[1])):
            par[k, sl, :] = val

    wr, wl = _iota((T, LANES), 0), _iota((T, LANES), 1)
    second = wr >= T // 2
    kk = 2 * jnp.where(second, wr - T // 2, wr)
    ii = jnp.where(second, wl - T, wl)
    mine = (ii >= 0) & (ii < T)
    tmask[...] = (jnp.where(mine & (ii + kk >= T - 1), 0xFFFF, 0)
                  | jnp.where(mine & (ii + kk + 1 >= T - 1), -0x10000, 0))
    hr, hl = _iota((T // 2, LANES), 0), _iota((T // 2, LANES), 1)
    tidx[...] = (hl + 2 * hr + (LANES - (T - 1))) & (LANES - 1)

    cp_u.wait()
    flip = (_iota((T, T), 0) + _iota((T, T), 1) == T - 1).astype(F32).astype(BF16)

    def to_lanes(c, carry):
        r = _mm(flip, u_v[pl.ds(pl.multiple_of(c * T, T), T), :])
        for bp in range((nblk + 1) // 2):
            first = r[:, 2 * bp * LANES:(2 * bp + 1) * LANES]
            full = 2 * bp + 1 < nblk
            other = (r[:, (2 * bp + 1) * LANES:(2 * bp + 2) * LANES] if full
                     else pltpu.roll(first, T, 1))
            q = jnp.concatenate([first, other], axis=0).T
            for j in range(LANES // GP if full else LANES // GP // 2):
                ut[bp * (LANES // GP) + j, pl.ds(c, GP, stride=CP), :] = q[j * GP:(j + 1) * GP]
        return carry

    lax.fori_loop(0, NCH, to_lanes, 0)

    lo_half = _iota((NCH, LANES), 1) < T
    row0 = _iota((NCH, LANES), 0) == 0

    def chan_base(g):
        bp = g // (LANES // GP)
        d1 = bp * LANES + g * GP
        d2 = d1 + jnp.where(2 * bp + 1 < nblk, LANES, T)
        return pl.multiple_of(d1, GP), pl.multiple_of(d2, GP)

    def vander(d):
        vr = [pw_re[pl.ds(d, 8, stride=pp), :]]
        vi = [pw_im[pl.ds(d, 8, stride=pp), :]]
        for k in range(3):
            mr = par[2 * k, pl.ds(d, 1), :]
            mi = par[2 * k + 1, pl.ds(d, 1), :]
            new = [_cmul(a, b, mr, mi) for a, b in zip(vr, vi)]
            vr += [n[0] for n in new]
            vi += [n[1] for n in new]
        return jnp.concatenate([jnp.concatenate(vr, axis=0), jnp.concatenate(vi, axis=0)], axis=1)

    def stage_states(g, p):
        d1, d2 = chan_base(g)
        slot = g % RING
        wcat = jnp.concatenate([vander(d1 + p), vander(d2 + p)], axis=0).astype(BF16)
        vbuf[slot, p] = wcat
        uu = ut[g, pl.ds(p * CP, NCH), :]
        um = jnp.concatenate([jnp.where(lo_half, uu, 0.0), jnp.where(lo_half, 0.0, uu)], axis=0)
        s = _mm(um, wcat)
        for half in range(2):
            for part in range(2):
                sbuf[slot, 2 * half + part, pl.ds(p * CP, NCH), :] = (
                    s[half * NCH:(half + 1) * NCH, part * LANES:(part + 1) * LANES])

    def stage_scan(g, half):
        d = chan_base(g)[half]
        slot = g % RING
        er, ei, gr, gi = (par[6 + k, pl.ds(d, GP), :] for k in range(4))
        zbuf[slot, 2 * half, pl.ds(0, GP, stride=CP), :] = par[10, pl.ds(d, GP), :]
        zbuf[slot, 2 * half + 1, pl.ds(0, GP, stride=CP), :] = par[11, pl.ds(d, GP), :]
        zr = zn = None
        for c in range(NCH - 1):
            sr = sbuf[slot, 2 * half, pl.ds(c, GP, stride=CP), :]
            si = sbuf[slot, 2 * half + 1, pl.ds(c, GP, stride=CP), :]
            tr, ti = _cmul(gr, gi, sr, si)
            if c == 0:
                zr, zn = tr, -ti
            else:
                zr, zn = er * zr + ei * zn + tr, er * zn - ei * zr - ti
            zbuf[slot, 2 * half, pl.ds(c + 1, GP, stride=CP), :] = zr
            zbuf[slot, 2 * half + 1, pl.ds(c + 1, GP, stride=CP), :] = zn

    def stage_readout(g, p):
        slot = g % RING
        z = jnp.concatenate(
            [jnp.concatenate([zbuf[slot, 2 * half + part, pl.ds(p * CP, NCH), :]
                              for part in range(2)], axis=1) for half in range(2)], axis=0)
        o = _mm_nt(z, vbuf[slot, p])
        y = jnp.where(lo_half, o[:NCH], o[NCH:])
        kbuf[slot, pl.ds(p, 1), :] = y[:1]
        ybuf[slot, p] = jnp.where(row0, 0.0, y)

    def pack_taps(g):
        bits = pltpu.bitcast(kbuf[g % RING].astype(BF16).astype(F32), I32)
        return lax.shift_right_logical(bits, 16) | pltpu.roll(bits, LANES - 1, 1)

    def stage_local(g, p, taps):
        slot = g % RING
        src = jnp.broadcast_to(taps[p:p + 1], (8, LANES))
        half = jnp.concatenate(
            [jnp.take_along_axis(src, tidx[pl.ds(8 * j, 8), :], axis=1)
             for j in range(T // 16)], axis=0)
        toe = pltpu.bitcast(jnp.concatenate([half, half], axis=0) & tmask[...], BF16)
        y2[g, pl.ds(p * CP, NCH), :] = _mm(ut[g, pl.ds(p * CP, NCH), :], toe) + ybuf[slot, p]

    def wave(i, live):
        taps = pack_taps(i - 3) if live[3] else None
        for p in range(GP):
            if live[3]:
                stage_local(i - 3, p, taps)
            if live[2]:
                stage_readout(i - 2, p)
            if live[1] and p % (GP // 2) == 0:
                stage_scan(i - 1, p // (GP // 2))
            if live[0]:
                stage_states(i, p)

    for i in range(3):
        wave(i, [i >= k for k in range(4)])

    def wave_body(i, carry):
        wave(i, [True] * 4)
        return carry

    lax.fori_loop(3, ngrp, wave_body, 0)
    for i in range(ngrp, ngrp + 3):
        wave(i, [i - k < ngrp for k in range(4)])

    dskip = dsk_ref[...].astype(F32).reshape(1, dm)
    lo_t = _iota((T, LANES), 1) < T

    def to_rows(c, carry):
        cols = []
        for bp in range((nblk + 1) // 2):
            full = 2 * bp + 1 < nblk
            parts = [y2[bp * (LANES // GP) + j, pl.ds(c, GP, stride=CP), :]
                     for j in range(LANES // GP if full else LANES // GP // 2)]
            q = jnp.concatenate(parts if full else parts + parts, axis=0).T
            cols += [q[:T], q[T:]] if full else [jnp.where(lo_t, q[:T], q[T:])]
        tsl = pl.ds(pl.multiple_of(c * T, T), T)
        y = jnp.concatenate(cols, axis=1) + u_v[tsl, :].astype(F32) * dskip
        oa_v[tsl, :] = y.astype(BF16)
        return carry

    lax.fori_loop(0, NCH, to_rows, 0)
    cp_oa.start()

    hp = heads // 2
    for i in range(3):
        cp_w[i].wait()
        words = raw_v.at[i].bitcast(U32)

        def relayout(b, carry, i=i, words=words):
            blk = words.at[pl.ds(pl.multiple_of(b * LANES * hp, LANES * hp), LANES * hp), :]
            dsl = pl.ds(pl.multiple_of(b * LANES, LANES), LANES)
            for j in range(hp):
                w = blk[pl.ds(j, LANES, stride=hp), :]
                wqkv_v[2 * j, dsl, i * dh:(i + 1) * dh] = pltpu.bitcast(w << 16, F32).astype(BF16)
                wqkv_v[2 * j + 1, dsl, i * dh:(i + 1) * dh] = pltpu.bitcast(
                    w & jnp.uint32(0xFFFF0000), F32).astype(BF16)
            return carry

        lax.fori_loop(0, nblk, relayout, 0)
    cp_x.wait()
    cp_wo.wait()

    qi, ki = _iota((rows, rows), 0), _iota((rows, rows), 1)
    visible = (qi < nmem) | (qi >= ki)
    scale = dh ** -0.5

    def out_copy(row):
        return pltpu.make_async_copy(ob_v.at[pl.ds(row, seg), :],
                                     out_hbm.at[pl.ds(row, seg), pl.ds(dm, dm)], sems.at[7])

    def segment(s, mem):
        row = pl.multiple_of(s * seg, seg)
        h = jnp.concatenate([mem, x_v[pl.ds(row, seg), :].astype(F32)], axis=0)
        st = {}
        acc = None
        wo_next = 0
        for i in range(heads + SKEW[3]):
            j = i - SKEW[3]
            if 0 <= j < heads:
                o, l = st.pop(("o", j))
                obuf[:, j * dh:(j + 1) * dh] = o * pltpu.reciprocal(l, approx=True)
            j = i - SKEW[2]
            if 0 <= j < heads:
                sc, m, v = st.pop(("m", j))
                e = jnp.exp(sc - m)
                st[("o", j)] = (_mm(e, v), jnp.sum(e, axis=-1, keepdims=True))
            j = i - SKEW[1]
            if 0 <= j < heads:
                sc, v = st.pop(("s", j))
                sc = jnp.where(visible, sc * scale, -1e9)
                st[("m", j)] = (sc, jnp.max(sc, axis=-1, keepdims=True), v)
            j = i - SKEW[0]
            if 0 <= j < heads:
                qkv = st.pop(("qkv", j))
                st[("s", j)] = (_mm_nt(qkv[:, :dh], qkv[:, dh:2 * dh]), qkv[:, 2 * dh:])
            if i < heads:
                st[("qkv", i)] = _mm(h, wqkv_v[i])
            else:
                stop = heads if i == heads + SKEW[3] - 1 else wo_next + 3
                part = _mm(obuf[:, wo_next * dh:stop * dh], wo_v[wo_next * dh:stop * dh, :])
                acc = part if acc is None else acc + part
                wo_next = stop
        ob_v[pl.ds(row, seg), :] = acc[nmem:].astype(BF16)
        out_copy(row).start()
        return acc[:nmem].astype(BF16).astype(F32)

    lax.fori_loop(0, seq // seg, segment, mem0_ref[...].astype(F32))
    cp_oa.wait()
    pltpu.make_async_copy(ob_v, out_hbm.at[:, pl.ds(dm, dm)], sems.at[7]).wait()


@functools.partial(jax.jit, static_argnames=("B_seg_len",))
def pallas_concat_heads__ssm_conv_s4__memory_aug_recurrent_mem_tr__prompt_kernel(
    A_u, A_A_re, A_A_im, A_B_re, A_B_im, A_C_re, A_C_im, A_log_dt, A_Dskip,
    B_x, B_mem0, B_Wq, B_Wk, B_Wv, B_Wo, B_seg_len,
):
    bsz, seq, dm = B_x.shape
    heads, dh = B_Wq.shape[1:]
    nmem = B_mem0.shape[1]
    seg = int(B_seg_len)
    assert bsz == 1 and A_u.shape == B_x.shape and A_A_re.shape == (dm, LANES)
    assert seq == NCH * T and seq % seg == 0 and seg % 16 == 0 and nmem % 8 == 0
    assert dh == LANES and dm % LANES == 0 and heads > 3 * SKEW[3]

    ngrp = dm // (2 * GP)
    hbm = pl.BlockSpec(memory_space=pl.ANY)
    vmem = pl.BlockSpec(memory_space=pltpu.VMEM)
    scratch = [
        pltpu.VMEM((seq, dm), BF16),
        pltpu.VMEM((seq, dm), BF16),
        pltpu.VMEM((3, dm * heads, dh), BF16),
        pltpu.VMEM((heads, dm, 3 * dh), BF16),
        pltpu.VMEM((heads * dh, dm), BF16),
        pltpu.VMEM((seq, dm), BF16),
        pltpu.VMEM((seq, dm), BF16),
        pltpu.VMEM((nmem + seg, heads * dh), F32),
        pltpu.VMEM((8 * (dm + 1), LANES), F32),
        pltpu.VMEM((8 * (dm + 1), LANES), F32),
        pltpu.VMEM((12, dm, LANES), F32),
        pltpu.VMEM((ngrp, GP * CP, LANES), F32),
        pltpu.VMEM((ngrp, GP * CP, LANES), F32),
        pltpu.VMEM((RING, GP, LANES, 2 * LANES), BF16),
        pltpu.VMEM((RING, 4, GP * CP, LANES), F32),
        pltpu.VMEM((RING, 4, GP * CP, LANES), F32),
        pltpu.VMEM((RING, GP, NCH, LANES), F32),
        pltpu.VMEM((RING, GP, LANES), F32),
        pltpu.VMEM((T, LANES), I32),
        pltpu.VMEM((T // 2, LANES), I32),
        pltpu.SemaphoreType.DMA((8,)),
    ]
    out = pl.pallas_call(
        functools.partial(_kernel, seq=seq, dm=dm, heads=heads, dh=dh, nmem=nmem, seg=seg),
        out_shape=jax.ShapeDtypeStruct((seq, 2 * dm), BF16),
        in_specs=[hbm] + [vmem] * 8 + [hbm, vmem, hbm, hbm, hbm, hbm],
        out_specs=hbm,
        scratch_shapes=scratch,
        compiler_params=pltpu.CompilerParams(vmem_limit_bytes=100 * 2**20),
        name="s4_rmt",
    )(A_u.reshape(seq, dm), A_A_re, A_A_im, A_B_re, A_B_im, A_C_re, A_C_im, A_log_dt, A_Dskip,
      B_x.reshape(seq, dm), B_mem0.reshape(nmem, dm),
      B_Wq.reshape(dm * heads, dh), B_Wk.reshape(dm * heads, dh), B_Wv.reshape(dm * heads, dh),
      B_Wo.reshape(heads * dh, dm))
    return out.reshape(bsz, seq, 2 * dm)
```

```python
import functools

import jax
import jax.numpy as jnp
from jax import lax
import jax.experimental.pallas as pl
import jax.experimental.pallas.tpu as pltpu

F32 = jnp.float32
BF16 = jnp.bfloat16
U32 = jnp.uint32
I32 = jnp.int32

LANES = 128
T = 64
NCH = 32
CP = NCH + 1
GP = 8
RING = 4
PRE = 8
UNROLL = 2
LAG = 2
SKEW = (2, 4, 6, 8)


def _mm(a, b):
    return lax.dot_general(a, b, (((1,), (0,)), ((), ())), preferred_element_type=F32)


def _mm_nt(a, b):
    return lax.dot_general(a, b, (((1,), (1,)), ((), ())), preferred_element_type=F32)


def _cmul(ar, ai, br, bi):
    return ar * br - ai * bi, ar * bi + ai * br


def _halves(x):
    return pltpu.bitcast(x, BF16)


def _iota(shape, dim):
    return lax.broadcasted_iota(I32, shape, dim)


def _kernel(u_hbm, are_ref, aim_ref, bre_ref, bim_ref, cre_ref, cim_ref, ldt_ref, dsk_ref,
            x_hbm, mem0_ref, wq_hbm, wk_hbm, wv_hbm, wo_hbm, out_hbm,
            u_v, x_v, raw_v, wqkv_v, wo_v, o_v, obuf,
            pw_re, pw_im, par, ut, y2, vbuf, sbuf, zbuf, ybuf, kbuf, pbuf, tbuf, tmask, tidx,
            u_sems, sems, *, seq, dm, heads, dh, nmem, seg):
    nblk = dm // LANES
    ngrp = dm // (2 * GP)
    pp = dm + 8
    rows = nmem + seg

    urows = seq // PRE

    def u_copy(i):
        sl = pl.ds(pl.multiple_of(i * urows, urows), urows)
        return pltpu.make_async_copy(u_hbm.at[sl, :], u_v.at[sl, :], u_sems.at[i])

    cp_w = [pltpu.make_async_copy(w, raw_v.at[i], sems.at[i])
            for i, w in enumerate((wq_hbm, wk_hbm, wv_hbm))]
    cp_x = pltpu.make_async_copy(x_hbm, x_v, sems.at[3])
    cp_wo = [pltpu.make_async_copy(wo_hbm.at[:, pl.ds(b * LANES, LANES)],
                                   wo_v.bitcast(BF16).at[b], sems.at[5 + b])
             for b in range(nblk)]
    for i in range(PRE):
        u_copy(i).start()
    cp_w[0].start()

    dt_row = jnp.exp(ldt_ref[...].astype(F32)).astype(BF16).astype(F32).reshape(1, dm)
    for b in range(nblk):
        par[0, pl.ds(b * LANES, LANES), :] = jnp.broadcast_to(
            dt_row[:, b * LANES:(b + 1) * LANES], (LANES, LANES)).T

    def mode_tables(r0, n):
        sl = pl.ds(r0, n)
        dt = par[0, sl, :]
        ar = dt * are_ref[sl, :].astype(F32)
        ai = dt * aim_ref[sl, :].astype(F32)
        mag = jnp.exp(ar)
        e1 = (mag * jnp.cos(ai), mag * jnp.sin(ai))
        w = _cmul(cre_ref[sl, :].astype(F32), cim_ref[sl, :].astype(F32),
                  dt * bre_ref[sl, :].astype(F32), dt * bim_ref[sl, :].astype(F32))
        g = _cmul(*w, *e1)
        e2 = _cmul(*e1, *e1)
        e4 = _cmul(*e2, *e2)
        e6 = _cmul(*e4, *e2)
        e8 = _cmul(*e4, *e4)
        even = [(jnp.ones_like(ar), jnp.zeros_like(ar)), e2, e4, e6, e8,
                _cmul(*e8, *e2), _cmul(*e8, *e4), _cmul(*e8, *e6)]
        for k, (pr, pi) in enumerate(even):
            pw_re[k, sl, :] = pr
            pw_im[k, sl, :] = pi
        e16 = _cmul(*e8, *e8)
        e32 = _cmul(*e16, *e16)
        e64 = _cmul(*e32, *e32)
        for k, val in enumerate((*e16, *e32, *e1, *e64, *g, w[0], -w[1])):
            par[k, sl, :] = val

    wr, wl = _iota((T, LANES), 0), _iota((T, LANES), 1)
    second = wr >= T // 2
    kk = 2 * jnp.where(second, wr - T // 2, wr)
    ii = jnp.where(second, wl - T, wl)
    mine = (ii >= 0) & (ii < T)
    tmask[...] = (jnp.where(mine & (ii + kk >= T - 1), 0xFFFF, 0)
                  | jnp.where(mine & (ii + kk + 1 >= T - 1), -0x10000, 0))
    hr, hl = _iota((T // 2, LANES), 0), _iota((T // 2, LANES), 1)
    tidx[...] = (hl + 2 * hr + (LANES - (T - 1))) & (LANES - 1)

    flip = (_iota((T, T), 0) + _iota((T, T), 1) == T - 1).astype(F32).astype(BF16)

    def to_lanes(c, r):
        for bp in range((nblk + 1) // 2):
            first = r[:, 2 * bp * LANES:(2 * bp + 1) * LANES]
            full = 2 * bp + 1 < nblk
            other = (r[:, (2 * bp + 1) * LANES:(2 * bp + 2) * LANES] if full
                     else pltpu.roll(first, T, 1))
            q = jnp.concatenate([first, other], axis=0).T
            for j in range(LANES // GP if full else LANES // GP // 2):
                ut[bp * (LANES // GP) + j, pl.ds(c, GP, stride=CP), :] = q[j * GP:(j + 1) * GP]

    def prepare(i, carry):
        u_copy(i).wait()
        per = NCH // PRE
        rev = [_mm(flip, u_v[pl.ds(pl.multiple_of((i * per + k) * T, T), T), :])
               for k in range(per)]
        n = dm // PRE
        for k in range(n // 16):
            mode_tables(pl.multiple_of(i * n + 16 * k, 16), 16)
            if k < per:
                to_lanes(i * per + k, rev[k])
        return carry

    lax.fori_loop(0, PRE, prepare, 0)

    lo_half = _iota((NCH, LANES), 1) < T
    row0 = _iota((NCH, LANES), 0) == 0

    def chan_base(g):
        bp = g // (LANES // GP)
        d1 = bp * LANES + g * GP
        d2 = d1 + jnp.where(2 * bp + 1 < nblk, LANES, T)
        return pl.multiple_of(d1, GP), pl.multiple_of(d2, GP)

    def vander(d):
        vr = [pw_re.reshape(8 * pp, LANES)[pl.ds(d, 8, stride=pp), :]]
        vi = [pw_im.reshape(8 * pp, LANES)[pl.ds(d, 8, stride=pp), :]]
        for k in range(3):
            mr = par[2 * k, pl.ds(d, 1), :]
            mi = par[2 * k + 1, pl.ds(d, 1), :]
            new = [_cmul(a, b, mr, mi) for a, b in zip(vr, vi)]
            vr += [n[0] for n in new]
            vi += [n[1] for n in new]
        return [pltpu.pack_elementwise(
            [jnp.concatenate(v[:4], axis=0), jnp.concatenate(v[4:], axis=0)], packed_dtype=BF16)
            for v in (vr, vi)]

    def prow(p):
        return pl.ds(p * CP, NCH)

    def states_issue(g, p):
        d1, d2 = chan_base(g)
        tiles = [jnp.concatenate(t, axis=0) for t in zip(vander(d1 + p), vander(d2 + p))]
        vbuf[g % RING, p, 0] = tiles[0]
        vbuf[g % RING, p, 1] = tiles[1]
        uu = ut[g, prow(p), :]
        um = jnp.concatenate([jnp.where(lo_half, uu, 0.0), jnp.where(lo_half, 0.0, uu)], axis=0)
        return _mm(um, jnp.concatenate([_halves(t) for t in tiles], axis=1))

    def states_store(g, p, s):
        for half in range(2):
            for part in range(2):
                sbuf[g % RING, 2 * half + part, prow(p), :] = (
                    s[half * NCH:(half + 1) * NCH, part * LANES:(part + 1) * LANES])

    def scan_steps(g, half):
        d = chan_base(g)[half]
        slot = g % RING
        er, ei, gr, gi = (par[6 + k, pl.ds(d, GP), :] for k in range(4))
        zbuf[slot, 2 * half, pl.ds(0, GP, stride=CP), :] = par[10, pl.ds(d, GP), :]
        zbuf[slot, 2 * half + 1, pl.ds(0, GP, stride=CP), :] = par[11, pl.ds(d, GP), :]
        zr = zn = None
        for c in range(NCH - 1):
            sr = sbuf[slot, 2 * half, pl.ds(c, GP, stride=CP), :]
            si = sbuf[slot, 2 * half + 1, pl.ds(c, GP, stride=CP), :]
            tr, ti = _cmul(gr, gi, sr, si)
            if c == 0:
                zr, zn = tr, -ti
            else:
                zr, zn = er * zr + ei * zn + tr, er * zn - ei * zr - ti
            zbuf[slot, 2 * half, pl.ds(c + 1, GP, stride=CP), :] = zr
            zbuf[slot, 2 * half + 1, pl.ds(c + 1, GP, stride=CP), :] = zn
            yield

    def readout_issue(g, p):
        slot = g % RING
        z = jnp.concatenate(
            [jnp.concatenate([zbuf[slot, 2 * half + part, prow(p), :] for part in range(2)], axis=1)
             for half in range(2)], axis=0)
        return _mm_nt(z, jnp.concatenate([_halves(vbuf[slot, p, t]) for t in range(2)], axis=1))

    def readout_store(g, p, o):
        slot = g % RING
        y = jnp.where(lo_half, o[:NCH], o[NCH:])
        kbuf[slot, pl.ds(p, 1), :] = y[:1]
        ybuf[slot, p] = jnp.where(row0, 0.0, y)

    def pack_taps(g):
        slot = g % RING
        bits = pltpu.bitcast(kbuf[slot].astype(BF16).astype(F32), I32)
        pbuf[slot] = lax.shift_right_logical(bits, 16) | pltpu.roll(bits, LANES - 1, 1)

    def local_gather(g, p):
        src = jnp.broadcast_to(pbuf[g % RING, pl.ds(p, 1), :], (8, LANES))
        return jnp.concatenate(
            [jnp.take_along_axis(src, tidx[pl.ds(8 * j, 8), :], axis=1) for j in range(T // 16)],
            axis=0)

    def local_mask(g, p, half):
        tbuf[g % RING, p] = jnp.concatenate([half, half], axis=0) & tmask[...]

    def local_issue(g, p):
        return _mm(ut[g, prow(p), :], _halves(tbuf[g % RING, p]))

    def local_store(g, p, y):
        y2[g, prow(p), :] = y + ybuf[g % RING, p]

    def wave(i, live):
        slots = GP + LAG
        scans = [scan_steps(i - 1, half) for half in range(2)] if live[1] else []
        st = {}
        if live[3]:
            pack_taps(i - 3)
        for p in range(slots):
            q = p - LAG
            if live[0] and 0 <= q < GP:
                states_store(i, q, st.pop(("s", q)))
            if live[2] and 0 <= q < GP:
                readout_store(i - 2, q, st.pop(("r", q)))
            if live[3] and 0 <= q < GP:
                local_mask(i - 3, q, st.pop(("g", q)))
            if live[4] and 0 <= q < GP:
                local_store(i - 4, q, st.pop(("l", q)))
            if live[3] and p < GP:
                st[("g", p)] = local_gather(i - 3, p)
            if live[2] and p < GP:
                st[("r", p)] = readout_issue(i - 2, p)
            if live[4] and p < GP:
                st[("l", p)] = local_issue(i - 4, p)
            if live[0] and p < GP:
                st[("s", p)] = states_issue(i, p)
            for _ in range((NCH - 1) * p // slots, (NCH - 1) * (p + 1) // slots):
                for scan in scans:
                    next(scan)

    for i in range(4):
        wave(i, [i >= k for k in range(5)])

    def wave_body(i, carry):
        for at, copies in ((3, cp_w[1:2]), (9, cp_w[2:]), (14, cp_wo + [cp_x])):
            @pl.when(i == at)
            def _(copies=copies):
                for c in copies:
                    c.start()

        for k in range(UNROLL):
            wave(UNROLL * i + k, [True] * 5)
        return carry

    lax.fori_loop(4 // UNROLL, ngrp // UNROLL, wave_body, 0)
    for i in range(ngrp, ngrp + 4):
        wave(i, [i - k < ngrp for k in range(5)])

    dskip = dsk_ref[...].astype(F32).reshape(1, dm)
    lo_s = _iota((seg, LANES), 1) < T

    def skip_rows(s, row):
        per = T // seg
        cols = []
        for bp in range((nblk + 1) // 2):
            full = 2 * bp + 1 < nblk
            parts = [y2[bp * (LANES // GP) + j, pl.ds(s // per, GP, stride=CP), :]
                     for j in range(LANES // GP if full else LANES // GP // 2)]
            q = jnp.concatenate(parts if full else parts + parts, axis=0).T
            top, bot = q[:seg], q[T:T + seg]
            for k in range(1, per):
                top = jnp.where(s % per == k, q[k * seg:(k + 1) * seg], top)
                bot = jnp.where(s % per == k, q[T + k * seg:T + (k + 1) * seg], bot)
            cols += [top, bot] if full else [jnp.where(lo_s, top, bot)]
        return jnp.concatenate(cols, axis=1) + u_v[pl.ds(row, seg), :].astype(F32) * dskip

    hp = heads // 2
    for i in range(3):
        cp_w[i].wait()
        words = raw_v.at[i].bitcast(U32)

        def relayout(b, carry, i=i, words=words):
            blk = words.at[pl.ds(pl.multiple_of(b * LANES * hp, LANES * hp), LANES * hp), :]
            dsl = pl.ds(pl.multiple_of(b * LANES, LANES), LANES)
            for j in range(hp):
                w = blk[pl.ds(j, LANES, stride=hp), :]
                wqkv_v[i, 2 * j, dsl, :] = pltpu.bitcast(w << 16, F32).astype(BF16)
                wqkv_v[i, 2 * j + 1, dsl, :] = pltpu.bitcast(
                    w & jnp.uint32(0xFFFF0000), F32).astype(BF16)
            return carry

        lax.fori_loop(0, nblk, relayout, 0)
    cp_x.wait()
    for c in cp_wo:
        c.wait()

    qi, ki = _iota((rows, rows), 0), _iota((rows, rows), 1)
    visible = (qi < nmem) | (qi >= ki)
    scale = dh ** -0.5

    def out_copy(row):
        return pltpu.make_async_copy(o_v.at[pl.ds(row, seg), :], out_hbm.at[pl.ds(row, seg), :],
                                     sems.at[4])

    def segment(s, mem):
        row = pl.multiple_of(s * seg, seg)
        h = jnp.concatenate([mem, x_v[pl.ds(row, seg), :].astype(F32)], axis=0)
        st = {}
        acc = None
        wo_next = 0
        for i in range(heads + SKEW[3]):
            j = i - SKEW[3]
            if 0 <= j < heads:
                o, l = st.pop(("o", j))
                obuf[:, j * dh:(j + 1) * dh] = o * pltpu.reciprocal(l, approx=True)
            j = i - SKEW[2]
            if 0 <= j < heads:
                sc, m, v = st.pop(("m", j))
                e = jnp.exp(sc - m)
                st[("o", j)] = (_mm(e, v), jnp.sum(e, axis=-1, keepdims=True))
            j = i - SKEW[1]
            if 0 <= j < heads:
                sc, v = st.pop(("s", j))
                sc = jnp.where(visible, sc * scale, -1e9)
                st[("m", j)] = (sc, jnp.max(sc, axis=-1, keepdims=True), v)
            j = i - SKEW[0]
            if 0 <= j < heads:
                qkv = st.pop(("qkv", j))
                st[("s", j)] = (_mm_nt(qkv[:, :dh], qkv[:, dh:2 * dh]), qkv[:, 2 * dh:])
            if i < heads:
                st[("qkv", i)] = _mm(h, jnp.concatenate([wqkv_v[t, i] for t in range(3)], axis=1))
            else:
                stop = heads if i == heads + SKEW[3] - 1 else wo_next + 3
                part = _mm(obuf[:, wo_next * dh:stop * dh],
                           jnp.concatenate([_halves(wo_v[b, wo_next * dh // 2:stop * dh // 2, :])
                                            for b in range(nblk)], axis=1))
                acc = part if acc is None else acc + part
                wo_next = stop
            if i == heads // 2:
                o_v[pl.ds(row, seg), :dm] = skip_rows(s, row).astype(BF16)
        o_v[pl.ds(row, seg), dm:] = acc[nmem:].astype(BF16)
        out_copy(row).start()
        return acc[:nmem].astype(BF16).astype(F32)

    lax.fori_loop(0, seq // seg, segment, mem0_ref[...].astype(F32))
    pltpu.make_async_copy(o_v, out_hbm, sems.at[4]).wait()


@functools.partial(jax.jit, static_argnames=("B_seg_len",))
def pallas_concat_heads__ssm_conv_s4__memory_aug_recurrent_mem_tr__prompt_kernel(
    A_u, A_A_re, A_A_im, A_B_re, A_B_im, A_C_re, A_C_im, A_log_dt, A_Dskip,
    B_x, B_mem0, B_Wq, B_Wk, B_Wv, B_Wo, B_seg_len,
):
    bsz, seq, dm = B_x.shape
    heads, dh = B_Wq.shape[1:]
    nmem = B_mem0.shape[1]
    seg = int(B_seg_len)
    assert bsz == 1 and A_u.shape == B_x.shape and A_A_re.shape == (dm, LANES)
    assert seq == NCH * T and seq % seg == 0 and seg % 16 == 0 and T % seg == 0 and nmem % 8 == 0
    assert dh == LANES and dm % LANES == 0 and heads > 3 * SKEW[3]

    ngrp = dm // (2 * GP)
    hbm = pl.BlockSpec(memory_space=pl.ANY)
    vmem = pl.BlockSpec(memory_space=pltpu.VMEM)
    scratch = [
        pltpu.VMEM((seq, dm), BF16),
        pltpu.VMEM((seq, dm), BF16),
        pltpu.VMEM((3, dm * heads, dh), BF16),
        pltpu.VMEM((3, heads, dm, dh), BF16),
        pltpu.VMEM((dm // LANES, heads * dh // 2, LANES), I32),
        pltpu.VMEM((seq, 2 * dm), BF16),
        pltpu.VMEM((nmem + seg, heads * dh), F32),
        pltpu.VMEM((8, dm + 8, LANES), F32),
        pltpu.VMEM((8, dm + 8, LANES), F32),
        pltpu.VMEM((12, dm, LANES), F32),
        pltpu.VMEM((ngrp, GP * CP, LANES), F32),
        pltpu.VMEM((ngrp, GP * CP, LANES), F32),
        pltpu.VMEM((RING, GP, 2, T, LANES), I32),
        pltpu.VMEM((RING, 4, GP * CP, LANES), F32),
        pltpu.VMEM((RING, 4, GP * CP, LANES), F32),
        pltpu.VMEM((RING, GP, NCH, LANES), F32),
        pltpu.VMEM((RING, GP, LANES), F32),
        pltpu.VMEM((RING, GP, LANES), I32),
        pltpu.VMEM((RING, GP, T, LANES), I32),
        pltpu.VMEM((T, LANES), I32),
        pltpu.VMEM((T // 2, LANES), I32),
        pltpu.SemaphoreType.DMA((PRE,)),
        pltpu.SemaphoreType.DMA((5 + dm // LANES,)),
    ]
    out = pl.pallas_call(
        functools.partial(_kernel, seq=seq, dm=dm, heads=heads, dh=dh, nmem=nmem, seg=seg),
        out_shape=jax.ShapeDtypeStruct((seq, 2 * dm), BF16),
        in_specs=[hbm] + [vmem] * 8 + [hbm, vmem, hbm, hbm, hbm, hbm],
        out_specs=hbm,
        scratch_shapes=scratch,
        compiler_params=pltpu.CompilerParams(vmem_limit_bytes=100 * 2**20),
        name="s4_rmt",
    )(A_u.reshape(seq, dm), A_A_re, A_A_im, A_B_re, A_B_im, A_C_re, A_C_im, A_log_dt, A_Dskip,
      B_x.reshape(seq, dm), B_mem0.reshape(nmem, dm),
      B_Wq.reshape(dm * heads, dh), B_Wk.reshape(dm * heads, dh), B_Wv.reshape(dm * heads, dh),
      B_Wo.reshape(heads * dh, dm))
    return out.reshape(bsz, seq, 2 * dm)
```

```python
import functools

import jax
import jax.numpy as jnp
from jax import lax
import jax.experimental.pallas as pl
import jax.experimental.pallas.tpu as pltpu

F32 = jnp.float32
BF16 = jnp.bfloat16
U32 = jnp.uint32
I32 = jnp.int32

LANES = 128
T = 64
NCH = 32
CP = NCH + 1
GP = 8
RING = 4
PRE = 8
UNROLL = 2
WO_STEP = 3
SKIP_AT = 4
LAG = 2
SKEW = (3, 5, 7, 9)


def _mm(a, b):
    return lax.dot_general(a, b, (((1,), (0,)), ((), ())), preferred_element_type=F32)


def _mm_nt(a, b):
    return lax.dot_general(a, b, (((1,), (1,)), ((), ())), preferred_element_type=F32)


def _cmul(ar, ai, br, bi):
    return ar * br - ai * bi, ar * bi + ai * br


def _halves(x):
    return pltpu.bitcast(x, BF16)


def _iota(shape, dim):
    return lax.broadcasted_iota(I32, shape, dim)


def _kernel(u_hbm, are_hbm, aim_hbm, bre_hbm, bim_hbm, cre_hbm, cim_hbm, ldt_ref, dsk_ref,
            x_hbm, mem0_ref, wq_hbm, wk_hbm, wv_hbm, wo_hbm, out_hbm,
            u_v, x_v, modes_v, raw_v, wqkv_v, wo_v, o_v, obuf,
            pw_re, pw_im, par, ut, y2, vbuf, sbuf, zbuf, ybuf, kbuf, pbuf, tbuf, tmask, tidx,
            u_sems, w_sems, wo_sems, sems, *, seq, dm, heads, dh, nmem, seg):
    nblk = dm // LANES
    ngrp = dm // (2 * GP)
    pp = dm + 8
    rows = nmem + seg

    def pre_copies(i):
        tsl = pl.ds(pl.multiple_of(i * (seq // PRE), seq // PRE), seq // PRE)
        dsl = pl.ds(pl.multiple_of(i * (dm // PRE), dm // PRE), dm // PRE)
        return [pltpu.make_async_copy(u_hbm.at[tsl, :], u_v.at[tsl, :], u_sems.at[i])] + [
            pltpu.make_async_copy(m.at[dsl, :], modes_v.at[k, dsl, :], u_sems.at[i])
            for k, m in enumerate((are_hbm, aim_hbm, bre_hbm, bim_hbm, cre_hbm, cim_hbm))]

    def pre_start(i):
        for c in pre_copies(i) + pre_copies(i + 1):
            c.start()

    wpitch = heads + 8

    def w_copy(t, r):
        src = (wq_hbm, wk_hbm, wv_hbm)[t].at[:, pl.ds(r * heads, heads), :]
        return pltpu.make_async_copy(src, raw_v.at[t, :, pl.ds(r * wpitch, heads), :], w_sems.at[t])

    def w_start(t, first=0):
        for r in range(first, 8):
            w_copy(t, r).start()

    def wo_copy(b):
        src = wo_hbm.at[:, pl.ds(pl.multiple_of(b * LANES, LANES), LANES)]
        return pltpu.make_async_copy(src, wo_v.bitcast(BF16).at[b], wo_sems.at[b])

    cp_x = pltpu.make_async_copy(x_hbm, x_v, sems.at[0])
    pre_start(0)

    dt_row = jnp.exp(ldt_ref[...].astype(F32)).astype(BF16).astype(F32).reshape(1, dm)
    for b in range(nblk):
        par[0, pl.ds(b * LANES, LANES), :] = jnp.broadcast_to(
            dt_row[:, b * LANES:(b + 1) * LANES], (LANES, LANES)).T

    def mode_tables(r0, n):
        sl = pl.ds(r0, n)
        dt = par[0, sl, :]
        a_re, a_im, b_re, b_im, c_re, c_im = (modes_v[k, sl, :].astype(F32) for k in range(6))
        ar = dt * a_re
        ai = dt * a_im
        mag = jnp.exp(ar)
        e1 = (mag * jnp.cos(ai), mag * jnp.sin(ai))
        w = _cmul(c_re, c_im, dt * b_re, dt * b_im)
        g = _cmul(*w, *e1)
        e2 = _cmul(*e1, *e1)
        e4 = _cmul(*e2, *e2)
        e6 = _cmul(*e4, *e2)
        e8 = _cmul(*e4, *e4)
        even = [(jnp.ones_like(ar), jnp.zeros_like(ar)), e2, e4, e6, e8,
                _cmul(*e8, *e2), _cmul(*e8, *e4), _cmul(*e8, *e6)]
        for k, (pr, pi) in enumerate(even[::-1]):
            pw_re[k, sl, :] = pr
            pw_im[k, sl, :] = pi
        e16 = _cmul(*e8, *e8)
        e32 = _cmul(*e16, *e16)
        e64 = _cmul(*e32, *e32)
        for k, val in enumerate((*e16, *e32, *e1, *e64, *g, w[0], -w[1])):
            par[k, sl, :] = val

    wr, wl = _iota((T, LANES), 0), _iota((T, LANES), 1)
    second = wr >= T // 2
    kk = 2 * jnp.where(second, wr - T // 2, wr)
    ii = jnp.where(second, wl - T, wl)
    mine = (ii >= 0) & (ii < T)
    tmask[...] = (jnp.where(mine & (ii + kk < T), 0xFFFF, 0)
                  | jnp.where(mine & (ii + kk + 1 < T), -0x10000, 0))
    hr, hl = _iota((T // 2, LANES), 0), _iota((T // 2, LANES), 1)
    tidx[...] = (hl + 2 * hr) & (LANES - 1)

    def to_lanes(c):
        tsl = pl.ds(pl.multiple_of(c * T, T), T)
        for bp in range((nblk + 1) // 2):
            first = u_v[tsl, pl.ds(2 * bp * LANES, LANES)]
            full = 2 * bp + 1 < nblk
            other = (u_v[tsl, pl.ds((2 * bp + 1) * LANES, LANES)] if full
                     else pltpu.roll(first, T, 1))
            q = jnp.concatenate([first, other], axis=0).T.astype(F32)
            for j in range(LANES // GP if full else LANES // GP // 2):
                ut[bp * (LANES // GP) + j, pl.ds(c, GP, stride=CP), :] = q[j * GP:(j + 1) * GP]

    def prepare(i, carry):
        for c in pre_copies(i):
            c.wait()
        pl.when(2 * i + 2 < PRE)(lambda: pre_start(2 * i + 2))
        for r in range(PRE // 2 + 1):
            pl.when(i == PRE // 2 - 1 + r)(w_copy(0, r).start)
        per = NCH // PRE
        n = dm // PRE
        for k in range(n // 16):
            mode_tables(pl.multiple_of(i * n + 16 * k, 16), 16)
            if k < per:
                to_lanes(i * per + k)
        return carry

    lax.fori_loop(0, PRE, prepare, 0)
    w_start(0, PRE // 2 + 1)

    lo_half = _iota((NCH, LANES), 1) < T
    row0 = _iota((NCH, LANES), 0) == 0

    def chan_base(g):
        bp = g // (LANES // GP)
        d1 = bp * LANES + g * GP
        d2 = d1 + jnp.where(2 * bp + 1 < nblk, LANES, T)
        return pl.multiple_of(d1, GP), pl.multiple_of(d2, GP)

    def vander(d):
        vr = [pw_re.reshape(8 * pp, LANES)[pl.ds(d, 8, stride=pp), :]]
        vi = [pw_im.reshape(8 * pp, LANES)[pl.ds(d, 8, stride=pp), :]]
        for k in range(3):
            mr = par[2 * k, pl.ds(d, 1), :]
            mi = par[2 * k + 1, pl.ds(d, 1), :]
            new = [_cmul(a, b, mr, mi) for a, b in zip(vr, vi)]
            vr = [n[0] for n in new] + vr
            vi = [n[1] for n in new] + vi
        return [pltpu.pack_elementwise(
            [jnp.concatenate(v[:4], axis=0), jnp.concatenate(v[4:], axis=0)], packed_dtype=BF16)
            for v in (vr, vi)]

    def prow(p):
        return pl.ds(p * CP, NCH)

    def states_issue(g, p):
        d1, d2 = chan_base(g)
        tiles = [jnp.concatenate(t, axis=0) for t in zip(vander(d1 + p), vander(d2 + p))]
        vbuf[g % RING, p, 0] = tiles[0]
        vbuf[g % RING, p, 1] = tiles[1]
        uu = ut[g, prow(p), :]
        um = jnp.concatenate([jnp.where(lo_half, uu, 0.0), jnp.where(lo_half, 0.0, uu)], axis=0)
        return _mm(um, jnp.concatenate([_halves(t) for t in tiles], axis=1))

    def states_store(g, p, s):
        for half in range(2):
            for part in range(2):
                sbuf[g % RING, 2 * half + part, prow(p), :] = (
                    s[half * NCH:(half + 1) * NCH, part * LANES:(part + 1) * LANES])

    def scan_steps(g, half):
        d = chan_base(g)[half]
        slot = g % RING
        er, ei, gr, gi = (par[6 + k, pl.ds(d, GP), :] for k in range(4))
        zbuf[slot, 2 * half, pl.ds(0, GP, stride=CP), :] = par[10, pl.ds(d, GP), :]
        zbuf[slot, 2 * half + 1, pl.ds(0, GP, stride=CP), :] = par[11, pl.ds(d, GP), :]
        zr = zn = None
        for c in range(NCH - 1):
            sr = sbuf[slot, 2 * half, pl.ds(c, GP, stride=CP), :]
            si = sbuf[slot, 2 * half + 1, pl.ds(c, GP, stride=CP), :]
            tr, ti = _cmul(gr, gi, sr, si)
            if c == 0:
                zr, zn = tr, -ti
            else:
                zr, zn = er * zr + ei * zn + tr, er * zn - ei * zr - ti
            zbuf[slot, 2 * half, pl.ds(c + 1, GP, stride=CP), :] = zr
            zbuf[slot, 2 * half + 1, pl.ds(c + 1, GP, stride=CP), :] = zn
            yield

    def readout_issue(g, p):
        slot = g % RING
        z = jnp.concatenate(
            [jnp.concatenate([zbuf[slot, 2 * half + part, prow(p), :] for part in range(2)], axis=1)
             for half in range(2)], axis=0)
        return _mm_nt(z, jnp.concatenate([_halves(vbuf[slot, p, t]) for t in range(2)], axis=1))

    def readout_store(g, p, o):
        slot = g % RING
        y = jnp.where(lo_half, o[:NCH], o[NCH:])
        kbuf[slot, pl.ds(p, 1), :] = y[:1]
        ybuf[slot, p] = jnp.where(row0, 0.0, y)

    def pack_taps(g):
        slot = g % RING
        bits = pltpu.bitcast(kbuf[slot].astype(BF16).astype(F32), I32)
        pbuf[slot] = lax.shift_right_logical(bits, 16) | pltpu.roll(bits, LANES - 1, 1)

    def local_gather(g, p):
        src = jnp.broadcast_to(pbuf[g % RING, pl.ds(p, 1), :], (8, LANES))
        return jnp.concatenate(
            [jnp.take_along_axis(src, tidx[pl.ds(8 * j, 8), :], axis=1) for j in range(T // 16)],
            axis=0)

    def local_mask(g, p, half):
        tbuf[g % RING, p] = jnp.concatenate([half, half], axis=0) & tmask[...]

    def local_issue(g, p):
        return _mm(ut[g, prow(p), :], _halves(tbuf[g % RING, p]))

    def local_store(g, p, y):
        y2[g, prow(p), :] = y + ybuf[g % RING, p]

    def wave(i, live):
        slots = GP + LAG
        scans = [scan_steps(i - 1, half) for half in range(2)] if live[1] else []
        st = {}
        if live[3]:
            pack_taps(i - 3)
        for p in range(slots):
            q = p - LAG
            if live[0] and 0 <= q < GP:
                states_store(i, q, st.pop(("s", q)))
            if live[2] and 0 <= q < GP:
                readout_store(i - 2, q, st.pop(("r", q)))
            if live[3] and 0 <= q < GP:
                local_mask(i - 3, q, st.pop(("g", q)))
            if live[4] and 0 <= q < GP:
                local_store(i - 4, q, st.pop(("l", q)))
            if live[3] and p < GP:
                st[("g", p)] = local_gather(i - 3, p)
            if live[2] and p < GP:
                st[("r", p)] = readout_issue(i - 2, p)
            if live[4] and p < GP:
                st[("l", p)] = local_issue(i - 4, p)
            if live[0] and p < GP:
                st[("s", p)] = states_issue(i, p)
            for _ in range((NCH - 1) * p // slots, (NCH - 1) * (p + 1) // slots):
                for scan in scans:
                    next(scan)

    for i in range(4):
        wave(i, [i >= k for k in range(5)])

    def wo_start():
        for b in range(nblk):
            wo_copy(b).start()

    def wave_body(i, carry):
        pl.when(i == 2)(lambda: w_start(1))
        pl.when(i == 7)(lambda: w_start(2))
        pl.when(i == 12)(wo_start)
        pl.when(i == 17)(cp_x.start)
        for k in range(UNROLL):
            wave(UNROLL * i + k, [True] * 5)
        return carry

    lax.fori_loop(4 // UNROLL, ngrp // UNROLL, wave_body, 0)
    for i in range(ngrp, ngrp + 4):
        wave(i, [i - k < ngrp for k in range(5)])

    dskip = dsk_ref[...].astype(F32).reshape(1, dm)
    lo_s = _iota((seg, LANES), 1) < T
    unflip = _iota((GP, LANES), 1) ^ (T - 1)

    def skip_rows(s, row, bp):
        per = T // seg
        full = 2 * bp + 1 < nblk
        parts = [jnp.take_along_axis(
            y2[bp * (LANES // GP) + j, pl.ds(s // per, GP, stride=CP), :], unflip, axis=1)
            for j in range(LANES // GP if full else LANES // GP // 2)]
        q = jnp.concatenate(parts if full else parts + parts, axis=0).T
        top, bot = q[:seg], q[T:T + seg]
        for k in range(1, per):
            top = jnp.where(s % per == k, q[k * seg:(k + 1) * seg], top)
            bot = jnp.where(s % per == k, q[T + k * seg:T + (k + 1) * seg], bot)
        for b, y in enumerate([top, bot] if full else [jnp.where(lo_s, top, bot)], 2 * bp):
            cols = pl.ds(b * LANES, LANES)
            y = y + u_v[pl.ds(row, seg), cols].astype(F32) * dskip[:, b * LANES:(b + 1) * LANES]
            o_v[pl.ds(row, seg), cols] = y.astype(BF16)

    words = raw_v.bitcast(U32)
    for t in range(3):
        for r in range(8):
            w_copy(t, r).wait()

        def relayout(b, carry, t=t):
            dsl = pl.ds(pl.multiple_of(b * LANES, LANES), LANES)
            for j in range(heads // 2):
                w = jnp.concatenate(
                    [words[t, b * (LANES // 8) + k, pl.ds(j, 8, stride=wpitch // 2), :]
                     for k in range(LANES // 8)], axis=0)
                wqkv_v[t, 2 * j, dsl, :] = pltpu.bitcast(w << 16, F32).astype(BF16)
                wqkv_v[t, 2 * j + 1, dsl, :] = pltpu.bitcast(
                    w & jnp.uint32(0xFFFF0000), F32).astype(BF16)
            return carry

        lax.fori_loop(0, nblk, relayout, 0)
    cp_x.wait()
    for b in range(nblk):
        wo_copy(b).wait()

    qi, ki = _iota((rows, rows), 0), _iota((rows, rows), 1)
    visible = (qi < nmem) | (qi >= ki)
    scale = dh ** -0.5

    def out_copy(row):
        return pltpu.make_async_copy(o_v.at[pl.ds(row, seg), :], out_hbm.at[pl.ds(row, seg), :],
                                     sems.at[1])

    def segment(s, mem):
        row = pl.multiple_of(s * seg, seg)
        h = jnp.concatenate([mem, x_v[pl.ds(row, seg), :].astype(F32)], axis=0)
        st = {}
        acc = None
        wo_next = 0
        for i in range(heads + SKEW[3]):
            j = i - SKEW[3]
            if 0 <= j < heads:
                o, l = st.pop(("o", j))
                obuf[:, j * dh:(j + 1) * dh] = o * pltpu.reciprocal(l, approx=True)
            j = i - SKEW[2]
            if 0 <= j < heads:
                sc, m, v = st.pop(("m", j))
                e = jnp.exp(sc - m)
                st[("o", j)] = (_mm(e, v), jnp.sum(e, axis=-1, keepdims=True))
            j = i - SKEW[1]
            if 0 <= j < heads:
                sc, v = st.pop(("s", j))
                sc = jnp.where(visible, sc * scale, -1e9)
                st[("m", j)] = (sc, jnp.max(sc, axis=-1, keepdims=True), v)
            j = i - SKEW[0]
            if 0 <= j < heads:
                qkv = st.pop(("qkv", j))
                st[("s", j)] = (_mm_nt(qkv[:, :dh], qkv[:, dh:2 * dh]), qkv[:, 2 * dh:])
            if i < heads:
                st[("qkv", i)] = _mm(h, jnp.concatenate([wqkv_v[t, i] for t in range(3)], axis=1))
            else:
                stop = heads if i == heads + SKEW[3] - 1 else min(wo_next + WO_STEP, i - SKEW[3] + 1)
                part = _mm(obuf[:, wo_next * dh:stop * dh],
                           jnp.concatenate([_halves(wo_v[b, wo_next * dh // 2:stop * dh // 2, :])
                                            for b in range(nblk)], axis=1))
                acc = part if acc is None else acc + part
                wo_next = stop
            if i % SKIP_AT == 0 and 0 < i // SKIP_AT <= (nblk + 1) // 2:
                skip_rows(s, row, i // SKIP_AT - 1)
        o_v[pl.ds(row, seg), dm:] = acc[nmem:].astype(BF16)
        out_copy(row).start()
        return acc[:nmem].astype(BF16).astype(F32)

    lax.fori_loop(0, seq // seg, segment, mem0_ref[...].astype(F32))
    pltpu.make_async_copy(o_v, out_hbm, sems.at[1]).wait()


@functools.partial(jax.jit, static_argnames=("B_seg_len",))
def pallas_concat_heads__ssm_conv_s4__memory_aug_recurrent_mem_tr__prompt_kernel(
    A_u, A_A_re, A_A_im, A_B_re, A_B_im, A_C_re, A_C_im, A_log_dt, A_Dskip,
    B_x, B_mem0, B_Wq, B_Wk, B_Wv, B_Wo, B_seg_len,
):
    bsz, seq, dm = B_x.shape
    heads, dh = B_Wq.shape[1:]
    nmem = B_mem0.shape[1]
    seg = int(B_seg_len)
    assert bsz == 1 and A_u.shape == B_x.shape and A_A_re.shape == (dm, LANES)
    assert seq == NCH * T and seq % seg == 0 and seg % 16 == 0 and T % seg == 0 and nmem % 8 == 0
    assert dh == LANES and dm % LANES == 0

    ngrp = dm // (2 * GP)
    hbm = pl.BlockSpec(memory_space=pl.ANY)
    vmem = pl.BlockSpec(memory_space=pltpu.VMEM)
    scratch = [
        pltpu.VMEM((seq, dm), BF16),
        pltpu.VMEM((seq, dm), BF16),
        pltpu.VMEM((6, dm, LANES), BF16),
        pltpu.VMEM((3, dm // 8, 8 * (heads + 8), dh), BF16),
        pltpu.VMEM((3, heads, dm, dh), BF16),
        pltpu.VMEM((dm // LANES, heads * dh // 2, LANES), I32),
        pltpu.VMEM((seq, 2 * dm), BF16),
        pltpu.VMEM((nmem + seg, heads * dh), F32),
        pltpu.VMEM((8, dm + 8, LANES), F32),
        pltpu.VMEM((8, dm + 8, LANES), F32),
        pltpu.VMEM((12, dm, LANES), F32),
        pltpu.VMEM((ngrp, GP * CP, LANES), F32),
        pltpu.VMEM((ngrp, GP * CP, LANES), F32),
        pltpu.VMEM((RING, GP, 2, T, LANES), I32),
        pltpu.VMEM((RING, 4, GP * CP, LANES), F32),
        pltpu.VMEM((RING, 4, GP * CP, LANES), F32),
        pltpu.VMEM((RING, GP, NCH, LANES), F32),
        pltpu.VMEM((RING, GP, LANES), F32),
        pltpu.VMEM((RING, GP, LANES), I32),
        pltpu.VMEM((RING, GP, T, LANES), I32),
        pltpu.VMEM((T, LANES), I32),
        pltpu.VMEM((T // 2, LANES), I32),
        pltpu.SemaphoreType.DMA((PRE,)),
        pltpu.SemaphoreType.DMA((3,)),
        pltpu.SemaphoreType.DMA((dm // LANES,)),
        pltpu.SemaphoreType.DMA((3,)),
    ]
    out = pl.pallas_call(
        functools.partial(_kernel, seq=seq, dm=dm, heads=heads, dh=dh, nmem=nmem, seg=seg),
        out_shape=jax.ShapeDtypeStruct((seq, 2 * dm), BF16),
        in_specs=[hbm] * 7 + [vmem, vmem, hbm, vmem] + [hbm] * 4,
        out_specs=hbm,
        scratch_shapes=scratch,
        compiler_params=pltpu.CompilerParams(vmem_limit_bytes=100 * 2**20),
        name="s4_rmt",
    )(A_u.reshape(seq, dm), A_A_re, A_A_im, A_B_re, A_B_im, A_C_re, A_C_im, A_log_dt, A_Dskip,
      B_x.reshape(seq, dm), B_mem0.reshape(nmem, dm),
      *(w.reshape(dm // 8, 8 * heads, dh) for w in (B_Wq, B_Wk, B_Wv)),
      B_Wo.reshape(heads * dh, dm))
    return out.reshape(bsz, seq, 2 * dm)
```

```python
import functools

import jax
import jax.numpy as jnp
from jax import lax
import jax.experimental.pallas as pl
import jax.experimental.pallas.tpu as pltpu

F32 = jnp.float32
BF16 = jnp.bfloat16
U32 = jnp.uint32
I32 = jnp.int32

LANES = 128
T = 64
NCH = 32
CP = NCH + 1
GP = 8
RING = 4
X_HEAD = 4
PRE = 4
STAGES = 5
ORDER = "SRGLgrlsz"
OFF = dict(s=0, r=0, g=0, l=0, S=2, R=2, G=2, L=2)
WO_STEP = 3
SKIP_AT = 4
SCAN = (3, 3, 3, 3, 3, 3, 3, 3, 3, 4)
LAG = 2
SKEW = (3, 5, 7, 9)


def _mm(a, b):
    return lax.dot_general(a, b, (((1,), (0,)), ((), ())), preferred_element_type=F32)


def _mm_nt(a, b):
    return lax.dot_general(a, b, (((1,), (1,)), ((), ())), preferred_element_type=F32)


def _cmul(ar, ai, br, bi):
    return ar * br - ai * bi, ar * bi + ai * br


def _halves(x):
    return pltpu.bitcast(x, BF16)


def _iota(shape, dim):
    return lax.broadcasted_iota(I32, shape, dim)


def _kernel(u_hbm, are_hbm, aim_hbm, bre_hbm, bim_hbm, cre_hbm, cim_hbm, ldt_ref, dsk_ref,
            x_hbm, mem0_ref, wq_hbm, wk_hbm, wv_hbm, wo_hbm, out_hbm,
            u_v, x_v, modes_v, raw_v, wqkv_v, wo_v, o_v, obuf,
            pw_re, pw_im, par, ut, y2, vbuf, sbuf, zbuf, ybuf, kbuf, pbuf, tbuf, tmask, tidx,
            u_sems, m_sems, w_sems, wo_sems, sems, *, seq, dm, heads, dh, nmem, seg):
    nblk = dm // LANES
    ngrp = dm // (2 * GP)
    pp = dm + 8
    rows = nmem + seg

    def mode_copies(b):
        dsl = pl.ds(pl.multiple_of(b * LANES, LANES), LANES)
        return [pltpu.make_async_copy(m.at[dsl, :], modes_v.at[k, dsl, :], m_sems.at[b])
                for k, m in enumerate((are_hbm, aim_hbm, bre_hbm, bim_hbm, cre_hbm, cim_hbm))]

    def mode_start(b):
        for c in mode_copies(b):
            c.start()

    def u_copy(i):
        tsl = pl.ds(pl.multiple_of(i * (seq // PRE), seq // PRE), seq // PRE)
        return pltpu.make_async_copy(u_hbm.at[tsl, :], u_v.at[tsl, :], u_sems.at[i])

    wpitch = heads + 8

    def w_copy(t, r):
        src = (wq_hbm, wk_hbm, wv_hbm)[t].at[:, pl.ds(r * heads, heads), :]
        return pltpu.make_async_copy(src, raw_v.at[t, :, pl.ds(r * wpitch, heads), :], w_sems.at[t])

    def w_start(t, first=0, stop=8):
        for r in range(first, stop):
            w_copy(t, r).start()

    def wo_copy(b):
        src = wo_hbm.at[:, pl.ds(pl.multiple_of(b * LANES, LANES), LANES)]
        return pltpu.make_async_copy(src, wo_v.bitcast(BF16).at[b], wo_sems.at[b])

    cp_x = [pltpu.make_async_copy(x_hbm.at[rs, :], x_v.at[rs, :], sems.at[k]) for k, rs in enumerate(
        (pl.ds(0, X_HEAD * seg), pl.ds(X_HEAD * seg, seq - X_HEAD * seg)))]
    mode_start(0)
    mode_start(1)
    u_copy(0).start()

    dt_row = jnp.exp(ldt_ref[...].astype(F32)).astype(BF16).astype(F32).reshape(1, dm)
    for b in range(nblk):
        par[0, pl.ds(b * LANES, LANES), :] = jnp.broadcast_to(
            dt_row[:, b * LANES:(b + 1) * LANES], (LANES, LANES)).T

    def mode_tables(r0, n):
        sl = pl.ds(r0, n)
        dt = par[0, sl, :]
        a_re, a_im, b_re, b_im, c_re, c_im = (modes_v[k, sl, :].astype(F32) for k in range(6))
        ar = dt * a_re
        ai = dt * a_im
        mag = jnp.exp(ar)
        e1 = (mag * jnp.cos(ai), mag * jnp.sin(ai))
        w = _cmul(c_re, c_im, dt * b_re, dt * b_im)
        g = _cmul(*w, *e1)
        e2 = _cmul(*e1, *e1)
        e4 = _cmul(*e2, *e2)
        e6 = _cmul(*e4, *e2)
        e8 = _cmul(*e4, *e4)
        even = [(jnp.ones_like(ar), jnp.zeros_like(ar)), e2, e4, e6, e8,
                _cmul(*e8, *e2), _cmul(*e8, *e4), _cmul(*e8, *e6)]
        for k, (pr, pi) in enumerate(even[::-1]):
            pw_re[k, sl, :] = pr
            pw_im[k, sl, :] = pi
        e16 = _cmul(*e8, *e8)
        e32 = _cmul(*e16, *e16)
        e64 = _cmul(*e32, *e32)
        for k, val in enumerate((*e16, *e32, *e1, *e64, *g, w[0], -w[1])):
            par[k, sl, :] = val

    wr, wl = _iota((T, LANES), 0), _iota((T, LANES), 1)
    second = wr >= T // 2
    kk = 2 * jnp.where(second, wr - T // 2, wr)
    ii = jnp.where(second, wl - T, wl)
    mine = (ii >= 0) & (ii < T)
    tmask[...] = (jnp.where(mine & (ii + kk < T), 0xFFFF, 0)
                  | jnp.where(mine & (ii + kk + 1 < T), -0x10000, 0))
    hr, hl = _iota((T // 2, LANES), 0), _iota((T // 2, LANES), 1)
    tidx[...] = (hl + 2 * hr) & (LANES - 1)

    def to_lanes(c):
        tsl = pl.ds(pl.multiple_of(c * T, T), T)
        for bp in range((nblk + 1) // 2):
            first = u_v[tsl, pl.ds(2 * bp * LANES, LANES)].astype(F32)
            full = 2 * bp + 1 < nblk
            other = (u_v[tsl, pl.ds((2 * bp + 1) * LANES, LANES)].astype(F32) if full
                     else pltpu.roll(first, T, 1))
            q = jnp.concatenate([first, other], axis=0).T
            for j in range(LANES // GP if full else LANES // GP // 2):
                ut[bp * (LANES // GP) + j, pl.ds(c, GP, stride=CP), :] = q[j * GP:(j + 1) * GP]

    def tables(b, carry):
        for c in mode_copies(b):
            c.wait()
        for k in range(LANES // 16):
            mode_tables(pl.multiple_of(b * LANES + 16 * k, 16), 16)
        pl.when(b + 2 < nblk)(lambda: mode_start(b + 2))
        pl.when(b + 1 < PRE)(lambda: u_copy(b + 1).start())
        return carry

    def prepare(i, carry):
        u_copy(i).wait()
        for k in range(NCH // PRE):
            to_lanes(i * (NCH // PRE) + k)
        for r in range(1, PRE):
            pl.when(i == r - 1)(lambda r=r: w_start(0, 2 * r, 2 * r + 2))
        return carry

    lax.fori_loop(0, nblk, tables, 0)
    w_start(0, 0, 2)
    lax.fori_loop(0, PRE, prepare, 0)

    lo_half = _iota((NCH, LANES), 1) < T
    row0 = _iota((NCH, LANES), 0) == 0

    def chan_base(g):
        bp = g // (LANES // GP)
        d1 = bp * LANES + g * GP
        d2 = d1 + jnp.where(2 * bp + 1 < nblk, LANES, T)
        return pl.multiple_of(d1, GP), pl.multiple_of(d2, GP)

    def vander(d):
        vr = [pw_re.reshape(8 * pp, LANES)[pl.ds(d, 8, stride=pp), :]]
        vi = [pw_im.reshape(8 * pp, LANES)[pl.ds(d, 8, stride=pp), :]]
        for k in range(3):
            mr = par[2 * k, pl.ds(d, 1), :]
            mi = par[2 * k + 1, pl.ds(d, 1), :]
            new = [_cmul(a, b, mr, mi) for a, b in zip(vr, vi)]
            vr = [n[0] for n in new] + vr
            vi = [n[1] for n in new] + vi
        return [pltpu.pack_elementwise(
            [jnp.concatenate(v[:4], axis=0), jnp.concatenate(v[4:], axis=0)], packed_dtype=BF16)
            for v in (vr, vi)]

    def prow(p):
        return pl.ds(p * CP, NCH)

    def states_issue(g, p):
        d1, d2 = chan_base(g)
        tiles = [jnp.concatenate(t, axis=0) for t in zip(vander(d1 + p), vander(d2 + p))]
        vbuf[g % RING, p, 0] = tiles[0]
        vbuf[g % RING, p, 1] = tiles[1]
        uu = ut[g, prow(p), :]
        um = jnp.concatenate([jnp.where(lo_half, uu, 0.0), jnp.where(lo_half, 0.0, uu)], axis=0)
        return _mm(um, jnp.concatenate([_halves(t) for t in tiles], axis=1))

    def states_store(g, p, s):
        for half in range(2):
            for part in range(2):
                sbuf[g % RING, 2 * half + part, prow(p), :] = (
                    s[half * NCH:(half + 1) * NCH, part * LANES:(part + 1) * LANES])

    def scan_steps(g, half):
        d = chan_base(g)[half]
        slot = g % RING
        er, ei, gr, gi = (par[6 + k, pl.ds(d, GP), :] for k in range(4))
        zbuf[slot, 2 * half, pl.ds(0, GP, stride=CP), :] = par[10, pl.ds(d, GP), :]
        zbuf[slot, 2 * half + 1, pl.ds(0, GP, stride=CP), :] = par[11, pl.ds(d, GP), :]
        zr = zn = None
        for c in range(NCH - 1):
            sr = sbuf[slot, 2 * half, pl.ds(c, GP, stride=CP), :]
            si = sbuf[slot, 2 * half + 1, pl.ds(c, GP, stride=CP), :]
            tr, ti = _cmul(gr, gi, sr, si)
            if c == 0:
                zr, zn = tr, -ti
            else:
                zr, zn = er * zr + ei * zn + tr, er * zn - ei * zr - ti
            zbuf[slot, 2 * half, pl.ds(c + 1, GP, stride=CP), :] = zr
            zbuf[slot, 2 * half + 1, pl.ds(c + 1, GP, stride=CP), :] = zn
            yield

    def readout_issue(g, p):
        slot = g % RING
        z = jnp.concatenate(
            [jnp.concatenate([zbuf[slot, 2 * half + part, prow(p), :] for part in range(2)], axis=1)
             for half in range(2)], axis=0)
        return _mm_nt(z, jnp.concatenate([_halves(vbuf[slot, p, t]) for t in range(2)], axis=1))

    def readout_store(g, p, o):
        slot = g % RING
        y = jnp.where(lo_half, o[:NCH], o[NCH:])
        kbuf[slot, pl.ds(p, 1), :] = y[:1]
        ybuf[slot, p] = jnp.where(row0, 0.0, y)

    def pack_taps(g):
        slot = g % RING
        bits = pltpu.bitcast(kbuf[slot].astype(BF16).astype(F32), I32)
        pbuf[slot] = lax.shift_right_logical(bits, 16) | pltpu.roll(bits, LANES - 1, 1)

    def local_gather(g, p):
        src = jnp.broadcast_to(pbuf[g % RING, pl.ds(p, 1), :], (8, LANES))
        return jnp.concatenate(
            [jnp.take_along_axis(src, tidx[pl.ds(8 * j, 8), :], axis=1) for j in range(T // 16)],
            axis=0)

    def local_mask(g, p, half):
        tbuf[g % RING, p] = jnp.concatenate([half, half], axis=0) & tmask[...]

    def local_issue(g, p):
        return _mm(ut[g, prow(p), :], _halves(tbuf[g % RING, p]))

    def local_store(g, p, y):
        y2[g, prow(p), :] = y + ybuf[g % RING, p]

    def wave(i, live):
        scans = [scan_steps(i - 1, half) for half in range(2)] if live[1] else []
        st = {}
        if live[3]:
            pack_taps(i - 3)
        stages = {"s": (0, states_issue, states_store), "r": (2, readout_issue, readout_store),
                  "g": (3, local_gather, local_mask), "l": (4, local_issue, local_store)}
        for p in range(len(SCAN)):
            for op in ORDER:
                if op == "z":
                    for _ in range(SCAN[p]):
                        for scan in scans:
                            next(scan)
                    continue
                k, issue, finish = stages[op.lower()]
                q = p - OFF[op]
                if live[k] and 0 <= q < GP:
                    if op.islower():
                        st[op, q] = issue(i - k, q)
                    else:
                        finish(i - k, q, st.pop((op.lower(), q)))
        assert not st

    for i in range(STAGES - 1):
        wave(i, [i >= k for k in range(STAGES)])

    def wo_start():
        for b in range(nblk):
            wo_copy(b).start()

    def wave_body(i, carry):
        pl.when(i == 4)(lambda: w_start(1))
        pl.when(i == 14)(lambda: w_start(2))
        pl.when(i == 24)(wo_start)
        pl.when(i == 24)(cp_x[0].start)
        wave(i, [True] * STAGES)
        return carry

    lax.fori_loop(STAGES - 1, ngrp, wave_body, 0)
    for i in range(ngrp, ngrp + STAGES - 1):
        wave(i, [i - k < ngrp for k in range(STAGES)])

    dskip = dsk_ref[...].astype(F32).reshape(1, dm)
    lo_s = _iota((seg, LANES), 1) < T
    unflip = _iota((GP, LANES), 1) ^ (T - 1)

    def skip_rows(s, row, bp):
        per = T // seg
        full = 2 * bp + 1 < nblk
        parts = [jnp.take_along_axis(
            y2[bp * (LANES // GP) + j, pl.ds(s // per, GP, stride=CP), :], unflip, axis=1)
            for j in range(LANES // GP if full else LANES // GP // 2)]
        q = jnp.concatenate(parts if full else parts + parts, axis=0).T
        top, bot = q[:seg], q[T:T + seg]
        for k in range(1, per):
            top = jnp.where(s % per == k, q[k * seg:(k + 1) * seg], top)
            bot = jnp.where(s % per == k, q[T + k * seg:T + (k + 1) * seg], bot)
        for b, y in enumerate([top, bot] if full else [jnp.where(lo_s, top, bot)], 2 * bp):
            cols = pl.ds(b * LANES, LANES)
            y = y + u_v[pl.ds(row, seg), cols].astype(F32) * dskip[:, b * LANES:(b + 1) * LANES]
            o_v[pl.ds(row, seg), cols] = y.astype(BF16)

    words = raw_v.bitcast(U32)
    for t in range(3):
        for r in range(8):
            w_copy(t, r).wait()

        def relayout(b, carry, t=t):
            dsl = pl.ds(pl.multiple_of(b * LANES, LANES), LANES)
            for j in range(heads // 2):
                w = jnp.concatenate(
                    [words[t, b * (LANES // 8) + k, pl.ds(j, 8, stride=wpitch // 2), :]
                     for k in range(LANES // 8)], axis=0)
                wqkv_v[t, 2 * j, dsl, :] = pltpu.bitcast(w << 16, F32).astype(BF16)
                wqkv_v[t, 2 * j + 1, dsl, :] = pltpu.bitcast(
                    w & jnp.uint32(0xFFFF0000), F32).astype(BF16)
            return carry

        lax.fori_loop(0, nblk, relayout, 0)
    cp_x[0].wait()
    for b in range(nblk):
        wo_copy(b).wait()

    cp_x[1].start()

    qi, ki = _iota((rows, rows), 0), _iota((rows, rows), 1)
    visible = (qi < nmem) | (qi >= ki)
    scale = dh ** -0.5

    def out_copy(row):
        return pltpu.make_async_copy(o_v.at[pl.ds(row, seg), :], out_hbm.at[pl.ds(row, seg), :],
                                     sems.at[2])

    def segment(s, mem):
        pl.when(s == X_HEAD)(cp_x[1].wait)
        row = pl.multiple_of(s * seg, seg)
        h = jnp.concatenate([mem, x_v[pl.ds(row, seg), :].astype(F32)], axis=0)
        st = {}
        acc = None
        wo_next = 0
        for i in range(heads + SKEW[3]):
            j = i - SKEW[3]
            if 0 <= j < heads:
                o, l = st.pop(("o", j))
                obuf[:, j * dh:(j + 1) * dh] = o * pltpu.reciprocal(l, approx=True)
            j = i - SKEW[2]
            if 0 <= j < heads:
                sc, m, v = st.pop(("m", j))
                e = jnp.exp(sc - m)
                st[("o", j)] = (_mm(e, v), jnp.sum(e, axis=-1, keepdims=True))
            j = i - SKEW[1]
            if 0 <= j < heads:
                sc, v = st.pop(("s", j))
                sc = jnp.where(visible, sc * scale, -1e9)
                st[("m", j)] = (sc, jnp.max(sc, axis=-1, keepdims=True), v)
            j = i - SKEW[0]
            if 0 <= j < heads:
                qkv = st.pop(("qkv", j))
                st[("s", j)] = (_mm_nt(qkv[:, :dh], qkv[:, dh:2 * dh]), qkv[:, 2 * dh:])
            if i < heads:
                st[("qkv", i)] = _mm(h, jnp.concatenate([wqkv_v[t, i] for t in range(3)], axis=1))
            else:
                stop = heads if i == heads + SKEW[3] - 1 else min(wo_next + WO_STEP, i - SKEW[3] + 1)
                part = _mm(obuf[:, wo_next * dh:stop * dh],
                           jnp.concatenate([_halves(wo_v[b, wo_next * dh // 2:stop * dh // 2, :])
                                            for b in range(nblk)], axis=1))
                acc = part if acc is None else acc + part
                wo_next = stop
            if i % SKIP_AT == 0 and 0 < i // SKIP_AT <= (nblk + 1) // 2:
                skip_rows(s, row, i // SKIP_AT - 1)
        o_v[pl.ds(row, seg), dm:] = acc[nmem:].astype(BF16)
        out_copy(row).start()
        return acc[:nmem].astype(BF16).astype(F32)

    lax.fori_loop(0, seq // seg, segment, mem0_ref[...].astype(F32))
    pltpu.make_async_copy(o_v, out_hbm, sems.at[2]).wait()


@functools.partial(jax.jit, static_argnames=("B_seg_len",))
def pallas_concat_heads__ssm_conv_s4__memory_aug_recurrent_mem_tr__prompt_kernel(
    A_u, A_A_re, A_A_im, A_B_re, A_B_im, A_C_re, A_C_im, A_log_dt, A_Dskip,
    B_x, B_mem0, B_Wq, B_Wk, B_Wv, B_Wo, B_seg_len,
):
    bsz, seq, dm = B_x.shape
    heads, dh = B_Wq.shape[1:]
    nmem = B_mem0.shape[1]
    seg = int(B_seg_len)
    assert bsz == 1 and A_u.shape == B_x.shape and A_A_re.shape == (dm, LANES)
    assert seq == NCH * T and seq % seg == 0 and seg % 16 == 0 and T % seg == 0 and nmem % 8 == 0
    assert dh == LANES and dm % LANES == 0

    ngrp = dm // (2 * GP)
    hbm = pl.BlockSpec(memory_space=pl.ANY)
    vmem = pl.BlockSpec(memory_space=pltpu.VMEM)
    scratch = [
        pltpu.VMEM((seq, dm), BF16),
        pltpu.VMEM((seq, dm), BF16),
        pltpu.VMEM((6, dm, LANES), BF16),
        pltpu.VMEM((3, dm // 8, 8 * (heads + 8), dh), BF16),
        pltpu.VMEM((3, heads, dm, dh), BF16),
        pltpu.VMEM((dm // LANES, heads * dh // 2, LANES), I32),
        pltpu.VMEM((seq, 2 * dm), BF16),
        pltpu.VMEM((nmem + seg, heads * dh), F32),
        pltpu.VMEM((8, dm + 8, LANES), F32),
        pltpu.VMEM((8, dm + 8, LANES), F32),
        pltpu.VMEM((12, dm, LANES), F32),
        pltpu.VMEM((ngrp, GP * CP, LANES), F32),
        pltpu.VMEM((ngrp, GP * CP, LANES), F32),
        pltpu.VMEM((RING, GP, 2, T, LANES), I32),
        pltpu.VMEM((RING, 4, GP * CP, LANES), F32),
        pltpu.VMEM((RING, 4, GP * CP, LANES), F32),
        pltpu.VMEM((RING, GP, NCH, LANES), F32),
        pltpu.VMEM((RING, GP, LANES), F32),
        pltpu.VMEM((RING, GP, LANES), I32),
        pltpu.VMEM((RING, GP, T, LANES), I32),
        pltpu.VMEM((T, LANES), I32),
        pltpu.VMEM((T // 2, LANES), I32),
        pltpu.SemaphoreType.DMA((PRE,)),
        pltpu.SemaphoreType.DMA((dm // LANES,)),
        pltpu.SemaphoreType.DMA((3,)),
        pltpu.SemaphoreType.DMA((dm // LANES,)),
        pltpu.SemaphoreType.DMA((3,)),
    ]
    out = pl.pallas_call(
        functools.partial(_kernel, seq=seq, dm=dm, heads=heads, dh=dh, nmem=nmem, seg=seg),
        out_shape=jax.ShapeDtypeStruct((seq, 2 * dm), BF16),
        in_specs=[hbm] * 7 + [vmem, vmem, hbm, vmem] + [hbm] * 4,
        out_specs=hbm,
        scratch_shapes=scratch,
        compiler_params=pltpu.CompilerParams(vmem_limit_bytes=100 * 2**20),
        name="s4_rmt",
    )(A_u.reshape(seq, dm), A_A_re, A_A_im, A_B_re, A_B_im, A_C_re, A_C_im, A_log_dt, A_Dskip,
      B_x.reshape(seq, dm), B_mem0.reshape(nmem, dm),
      *(w.reshape(dm // 8, 8 * heads, dh) for w in (B_Wq, B_Wk, B_Wv)),
      B_Wo.reshape(heads * dh, dm))
    return out.reshape(bsz, seq, 2 * dm)
```

```python
import functools

import jax
import jax.numpy as jnp
from jax import lax
import jax.experimental.pallas as pl
import jax.experimental.pallas.tpu as pltpu

F32 = jnp.float32
BF16 = jnp.bfloat16
U32 = jnp.uint32
I32 = jnp.int32

LANES = 128
T = 64
NCH = 32
CP = NCH + 1
GP = 8
STAGES = 5
RING = 4
LAG = 2
PRE = 4
X_HEAD = 4
SKEW = (3, 5, 7, 9)
WO_STEP = 3
SKIP_AT = 4


def _mm(a, b):
    return lax.dot_general(a, b, (((1,), (0,)), ((), ())), preferred_element_type=F32)


def _mm_nt(a, b):
    return lax.dot_general(a, b, (((1,), (1,)), ((), ())), preferred_element_type=F32)


def _cmul(ar, ai, br, bi):
    return ar * br - ai * bi, ar * bi + ai * br


def _halves(x):
    return pltpu.bitcast(x, BF16)


def _iota(shape, dim):
    return lax.broadcasted_iota(I32, shape, dim)


def _kernel(u_hbm, are_hbm, aim_hbm, bre_hbm, bim_hbm, cre_hbm, cim_hbm, ldt_ref, dsk_ref,
            x_hbm, mem0_ref, wq_hbm, wk_hbm, wv_hbm, wo_hbm, out_hbm,
            u_v, x_v, modes_v, raw_v, wqkv_v, wo_v, o_v, obuf,
            pw_re, pw_im, par, ut, y2, vbuf, sbuf, zbuf, ybuf, kbuf, pbuf, tbuf, tmask, tidx,
            u_sems, m_sems, w_sems, sems, *, seq, dm, heads, dh, nmem, seg):
    nblk = dm // LANES
    ngrp = dm // (2 * GP)
    pp = dm + 8
    rows = nmem + seg

    def mode_copies(b):
        dsl = pl.ds(pl.multiple_of(b * LANES, LANES), LANES)
        return [pltpu.make_async_copy(m.at[dsl, :], modes_v.at[k, dsl, :], m_sems.at[b])
                for k, m in enumerate((are_hbm, aim_hbm, bre_hbm, bim_hbm, cre_hbm, cim_hbm))]

    def mode_start(b):
        for c in mode_copies(b):
            c.start()

    def u_copy(i):
        tsl = pl.ds(pl.multiple_of(i * (seq // PRE), seq // PRE), seq // PRE)
        return pltpu.make_async_copy(u_hbm.at[tsl, :], u_v.at[tsl, :], u_sems.at[i])

    wpitch = heads + 8

    def w_copy(t, r):
        src = (wq_hbm, wk_hbm, wv_hbm)[t].at[:, pl.ds(r * heads, heads), :]
        return pltpu.make_async_copy(src, raw_v.at[t, :, pl.ds(r * wpitch, heads), :], w_sems.at[t])

    def w_start(t, first=0, stop=8):
        for r in range(first, stop):
            w_copy(t, r).start()

    cp_wo = pltpu.make_async_copy(wo_hbm, wo_v, sems.at[3])
    cp_x = [pltpu.make_async_copy(x_hbm.at[rs, :], x_v.at[rs, :], sems.at[k]) for k, rs in enumerate(
        (pl.ds(0, X_HEAD * seg), pl.ds(X_HEAD * seg, seq - X_HEAD * seg)))]
    mode_start(0)
    mode_start(1)
    u_copy(0).start()

    dt_row = jnp.exp(ldt_ref[...].astype(F32)).astype(BF16).astype(F32).reshape(1, dm)
    for b in range(nblk):
        par[0, pl.ds(b * LANES, LANES), :] = jnp.broadcast_to(
            dt_row[:, b * LANES:(b + 1) * LANES], (LANES, LANES)).T

    def mode_tables(r0, n):
        sl = pl.ds(r0, n)
        dt = par[0, sl, :]
        a_re, a_im, b_re, b_im, c_re, c_im = (modes_v[k, sl, :].astype(F32) for k in range(6))
        ar = dt * a_re
        ai = dt * a_im
        mag = jnp.exp(ar)
        e1 = (mag * jnp.cos(ai), mag * jnp.sin(ai))
        w = _cmul(c_re, c_im, dt * b_re, dt * b_im)
        g = _cmul(*w, *e1)
        e2 = _cmul(*e1, *e1)
        e4 = _cmul(*e2, *e2)
        e6 = _cmul(*e4, *e2)
        e8 = _cmul(*e4, *e4)
        even = [(jnp.ones_like(ar), jnp.zeros_like(ar)), e2, e4, e6, e8,
                _cmul(*e8, *e2), _cmul(*e8, *e4), _cmul(*e8, *e6)]
        for k, (pr, pi) in enumerate(even[::-1]):
            pw_re[k, sl, :] = pr
            pw_im[k, sl, :] = pi
        e16 = _cmul(*e8, *e8)
        e32 = _cmul(*e16, *e16)
        e64 = _cmul(*e32, *e32)
        for k, val in enumerate((*e16, *e32, *e1, *e64, *g, w[0], -w[1])):
            par[k, sl, :] = val

    wr, wl = _iota((T, LANES), 0), _iota((T, LANES), 1)
    second = wr >= T // 2
    kk = 2 * jnp.where(second, wr - T // 2, wr)
    ii = jnp.where(second, wl - T, wl)
    mine = (ii >= 0) & (ii < T)
    tmask[...] = (jnp.where(mine & (ii + kk < T), 0xFFFF, 0)
                  | jnp.where(mine & (ii + kk + 1 < T), -0x10000, 0))
    hr, hl = _iota((T // 2, LANES), 0), _iota((T // 2, LANES), 1)
    tidx[...] = (hl + 2 * hr) & (LANES - 1)

    def to_lanes(c):
        tsl = pl.ds(pl.multiple_of(c * T, T), T)
        for bp in range((nblk + 1) // 2):
            first = u_v[tsl, pl.ds(2 * bp * LANES, LANES)].astype(F32)
            full = 2 * bp + 1 < nblk
            other = (u_v[tsl, pl.ds((2 * bp + 1) * LANES, LANES)].astype(F32) if full
                     else pltpu.roll(first, T, 1))
            q = jnp.concatenate([first, other], axis=0).T
            for j in range(LANES // GP if full else LANES // GP // 2):
                ut[bp * (LANES // GP) + j, pl.ds(c, GP, stride=CP), :] = q[j * GP:(j + 1) * GP]

    def tables(b, carry):
        for c in mode_copies(b):
            c.wait()
        for k in range(LANES // 16):
            mode_tables(pl.multiple_of(b * LANES + 16 * k, 16), 16)
        pl.when(b + 2 < nblk)(lambda: mode_start(b + 2))
        pl.when(b + 1 < PRE)(lambda: u_copy(b + 1).start())
        return carry

    def prepare(i, carry):
        u_copy(i).wait()
        for k in range(NCH // PRE):
            to_lanes(i * (NCH // PRE) + k)
        for r in range(1, PRE):
            pl.when(i == r - 1)(lambda r=r: w_start(0, 2 * r, 2 * r + 2))
        return carry

    lax.fori_loop(0, nblk, tables, 0)
    w_start(0, 0, 2)
    lax.fori_loop(0, PRE, prepare, 0)

    lo_half = _iota((NCH, LANES), 1) < T
    row0 = _iota((NCH, LANES), 0) == 0

    def chan_base(g):
        bp = g // (LANES // GP)
        d1 = bp * LANES + g * GP
        d2 = d1 + jnp.where(2 * bp + 1 < nblk, LANES, T)
        return pl.multiple_of(d1, GP), pl.multiple_of(d2, GP)

    def vander(d):
        vr = [pw_re.reshape(8 * pp, LANES)[pl.ds(d, 8, stride=pp), :]]
        vi = [pw_im.reshape(8 * pp, LANES)[pl.ds(d, 8, stride=pp), :]]
        for k in range(3):
            mr = par[2 * k, pl.ds(d, 1), :]
            mi = par[2 * k + 1, pl.ds(d, 1), :]
            new = [_cmul(a, b, mr, mi) for a, b in zip(vr, vi)]
            vr = [n[0] for n in new] + vr
            vi = [n[1] for n in new] + vi
        return [pltpu.pack_elementwise(
            [jnp.concatenate(v[:4], axis=0), jnp.concatenate(v[4:], axis=0)], packed_dtype=BF16)
            for v in (vr, vi)]

    def prow(p):
        return pl.ds(p * CP, NCH)

    def states_issue(g, p):
        d1, d2 = chan_base(g)
        tiles = [jnp.concatenate(t, axis=0) for t in zip(vander(d1 + p), vander(d2 + p))]
        vbuf[g % RING, p, 0] = tiles[0]
        vbuf[g % RING, p, 1] = tiles[1]
        uu = ut[g, prow(p), :]
        um = jnp.concatenate([jnp.where(lo_half, uu, 0.0), jnp.where(lo_half, 0.0, uu)], axis=0)
        return _mm(um, jnp.concatenate([_halves(t) for t in tiles], axis=1))

    def states_store(g, p, s):
        for half in range(2):
            for part in range(2):
                sbuf[g % RING, 2 * half + part, prow(p), :] = (
                    s[half * NCH:(half + 1) * NCH, part * LANES:(part + 1) * LANES])

    def scan_steps(g, half):
        d = chan_base(g)[half]
        slot = g % RING
        er, ei, gr, gi = (par[6 + k, pl.ds(d, GP), :] for k in range(4))
        zbuf[slot, 2 * half, pl.ds(0, GP, stride=CP), :] = par[10, pl.ds(d, GP), :]
        zbuf[slot, 2 * half + 1, pl.ds(0, GP, stride=CP), :] = par[11, pl.ds(d, GP), :]
        zr = zn = None
        for c in range(NCH - 1):
            sr = sbuf[slot, 2 * half, pl.ds(c, GP, stride=CP), :]
            si = sbuf[slot, 2 * half + 1, pl.ds(c, GP, stride=CP), :]
            tr, ti = _cmul(gr, gi, sr, si)
            if c == 0:
                zr, zn = tr, -ti
            else:
                zr, zn = er * zr + ei * zn + tr, er * zn - ei * zr - ti
            zbuf[slot, 2 * half, pl.ds(c + 1, GP, stride=CP), :] = zr
            zbuf[slot, 2 * half + 1, pl.ds(c + 1, GP, stride=CP), :] = zn
            yield

    def readout_issue(g, p):
        slot = g % RING
        z = jnp.concatenate(
            [jnp.concatenate([zbuf[slot, 2 * half + part, prow(p), :] for part in range(2)], axis=1)
             for half in range(2)], axis=0)
        return _mm_nt(z, jnp.concatenate([_halves(vbuf[slot, p, t]) for t in range(2)], axis=1))

    def readout_store(g, p, o):
        slot = g % RING
        y = jnp.where(lo_half, o[:NCH], o[NCH:])
        kbuf[slot, pl.ds(p, 1), :] = y[:1]
        ybuf[slot, p] = jnp.where(row0, 0.0, y)

    def pack_taps(g):
        slot = g % RING
        bits = pltpu.bitcast(kbuf[slot].astype(BF16).astype(F32), I32)
        pbuf[slot] = lax.shift_right_logical(bits, 16) | pltpu.roll(bits, LANES - 1, 1)

    def local_gather(g, p):
        src = jnp.broadcast_to(pbuf[g % RING, pl.ds(p, 1), :], (8, LANES))
        return jnp.concatenate(
            [jnp.take_along_axis(src, tidx[pl.ds(8 * j, 8), :], axis=1) for j in range(T // 16)],
            axis=0)

    def local_mask(g, p, half):
        tbuf[g % RING, p] = jnp.concatenate([half, half], axis=0) & tmask[...]

    def local_issue(g, p):
        return _mm(ut[g, prow(p), :], _halves(tbuf[g % RING, p]))

    def local_store(g, p, y):
        y2[g, prow(p), :] = y + ybuf[g % RING, p]

    def wave(i, live):
        states = (0, states_issue, states_store)
        readout = (2, readout_issue, readout_store)
        taps = (3, local_gather, local_mask)
        local = (4, local_issue, local_store)
        scans = [scan_steps(i - 1, half) for half in range(2)] if live[1] else []
        slots = GP + LAG
        pending = {}
        if live[3]:
            pack_taps(i - 3)
        for p in range(slots):
            for k, _, finish in (states, readout, taps, local):
                if live[k] and p >= LAG:
                    finish(i - k, p - LAG, pending.pop((k, p - LAG)))
            for k, issue, _ in (taps, readout, local, states):
                if live[k] and p < GP:
                    pending[k, p] = issue(i - k, p)
            for _ in range((NCH - 1) * p // slots, (NCH - 1) * (p + 1) // slots):
                for scan in scans:
                    next(scan)

    for i in range(STAGES - 1):
        wave(i, [i >= k for k in range(STAGES)])

    def wave_body(i, carry):
        pl.when(i == 4)(lambda: w_start(1))
        pl.when(i == 14)(lambda: w_start(2))
        pl.when(i == 24)(cp_wo.start)
        pl.when(i == 24)(cp_x[0].start)
        wave(i, [True] * STAGES)
        return carry

    lax.fori_loop(STAGES - 1, ngrp, wave_body, 0)
    for i in range(ngrp, ngrp + STAGES - 1):
        wave(i, [i - k < ngrp for k in range(STAGES)])

    dskip = dsk_ref[...].astype(F32).reshape(1, dm)
    lo_s = _iota((seg, LANES), 1) < T
    unflip = _iota((GP, LANES), 1) ^ (T - 1)

    def skip_rows(s, row, bp):
        per = T // seg
        full = 2 * bp + 1 < nblk
        parts = [jnp.take_along_axis(
            y2[bp * (LANES // GP) + j, pl.ds(s // per, GP, stride=CP), :], unflip, axis=1)
            for j in range(LANES // GP if full else LANES // GP // 2)]
        q = jnp.concatenate(parts if full else parts + parts, axis=0).T
        top, bot = q[:seg], q[T:T + seg]
        for k in range(1, per):
            top = jnp.where(s % per == k, q[k * seg:(k + 1) * seg], top)
            bot = jnp.where(s % per == k, q[T + k * seg:T + (k + 1) * seg], bot)
        for b, y in enumerate([top, bot] if full else [jnp.where(lo_s, top, bot)], 2 * bp):
            cols = pl.ds(b * LANES, LANES)
            y = y + u_v[pl.ds(row, seg), cols].astype(F32) * dskip[:, b * LANES:(b + 1) * LANES]
            o_v[pl.ds(row, seg), cols] = y.astype(BF16)

    words = raw_v.bitcast(U32)
    for t in range(3):
        for r in range(8):
            w_copy(t, r).wait()

        def relayout(b, carry, t=t):
            dsl = pl.ds(pl.multiple_of(b * LANES, LANES), LANES)
            for j in range(heads // 2):
                w = jnp.concatenate(
                    [words[t, b * (LANES // 8) + k, pl.ds(j, 8, stride=wpitch // 2), :]
                     for k in range(LANES // 8)], axis=0)
                wqkv_v[t, 2 * j, dsl, :] = pltpu.bitcast(w << 16, F32).astype(BF16)
                wqkv_v[t, 2 * j + 1, dsl, :] = pltpu.bitcast(
                    w & jnp.uint32(0xFFFF0000), F32).astype(BF16)
            return carry

        lax.fori_loop(0, nblk, relayout, 0)
    cp_x[0].wait()
    cp_wo.wait()

    cp_x[1].start()

    qi, ki = _iota((rows, rows), 0), _iota((rows, rows), 1)
    visible = (qi < nmem) | (qi >= ki)
    scale = dh ** -0.5

    def out_copy(row):
        return pltpu.make_async_copy(o_v.at[pl.ds(row, seg), :], out_hbm.at[pl.ds(row, seg), :],
                                     sems.at[2])

    def segment(s, mem):
        pl.when(s == X_HEAD)(cp_x[1].wait)
        row = pl.multiple_of(s * seg, seg)
        h = jnp.concatenate([mem, x_v[pl.ds(row, seg), :].astype(F32)], axis=0)
        st = {}
        acc = None
        wo_next = 0
        for i in range(heads + SKEW[3]):
            j = i - SKEW[3]
            if 0 <= j < heads:
                o, l = st.pop(("o", j))
                r = pltpu.reciprocal(l, approx=True)
                obuf[:, j * dh:(j + 1) * dh] = o * (r * (2.0 - l * r))
            j = i - SKEW[2]
            if 0 <= j < heads:
                sc, m, v = st.pop(("m", j))
                e = jnp.exp(sc - m)
                st[("o", j)] = (_mm(e, v), jnp.sum(e, axis=-1, keepdims=True))
            j = i - SKEW[1]
            if 0 <= j < heads:
                sc, v = st.pop(("s", j))
                sc = jnp.where(visible, sc * scale, -1e9)
                st[("m", j)] = (sc, jnp.max(sc, axis=-1, keepdims=True), v)
            j = i - SKEW[0]
            if 0 <= j < heads:
                qkv = st.pop(("qkv", j))
                st[("s", j)] = (_mm_nt(qkv[:, :dh], qkv[:, dh:2 * dh]), qkv[:, 2 * dh:])
            if i < heads:
                st[("qkv", i)] = _mm(h, jnp.concatenate([wqkv_v[t, i] for t in range(3)], axis=1))
            else:
                stop = heads if i == heads + SKEW[3] - 1 else min(wo_next + WO_STEP, i - SKEW[3] + 1)
                part = _mm(obuf[:, wo_next * dh:stop * dh], wo_v[wo_next * dh:stop * dh, :])
                acc = part if acc is None else acc + part
                wo_next = stop
            if i % SKIP_AT == 0 and 0 < i // SKIP_AT <= (nblk + 1) // 2:
                skip_rows(s, row, i // SKIP_AT - 1)
        o_v[pl.ds(row, seg), dm:] = acc[nmem:].astype(BF16)
        out_copy(row).start()
        return acc[:nmem].astype(BF16).astype(F32)

    lax.fori_loop(0, seq // seg, segment, mem0_ref[...].astype(F32))
    pltpu.make_async_copy(o_v, out_hbm, sems.at[2]).wait()


@functools.partial(jax.jit, static_argnames=("B_seg_len",))
def pallas_concat_heads__ssm_conv_s4__memory_aug_recurrent_mem_tr__prompt_kernel(
    A_u, A_A_re, A_A_im, A_B_re, A_B_im, A_C_re, A_C_im, A_log_dt, A_Dskip,
    B_x, B_mem0, B_Wq, B_Wk, B_Wv, B_Wo, B_seg_len,
):
    bsz, seq, dm = B_x.shape
    heads, dh = B_Wq.shape[1:]
    nmem = B_mem0.shape[1]
    seg = int(B_seg_len)
    assert bsz == 1 and A_u.shape == B_x.shape and A_A_re.shape == (dm, LANES)
    assert seq == NCH * T and seq % seg == 0 and seg % 16 == 0 and T % seg == 0 and nmem % 8 == 0
    assert dh == LANES and dm % LANES == 0

    ngrp = dm // (2 * GP)
    hbm = pl.BlockSpec(memory_space=pl.ANY)
    vmem = pl.BlockSpec(memory_space=pltpu.VMEM)
    scratch = [
        pltpu.VMEM((seq, dm), BF16),
        pltpu.VMEM((seq, dm), BF16),
        pltpu.VMEM((6, dm, LANES), BF16),
        pltpu.VMEM((3, dm // 8, 8 * (heads + 8), dh), BF16),
        pltpu.VMEM((3, heads, dm, dh), BF16),
        pltpu.VMEM((heads * dh, dm), BF16),
        pltpu.VMEM((seq, 2 * dm), BF16),
        pltpu.VMEM((nmem + seg, heads * dh), F32),
        pltpu.VMEM((8, dm + 8, LANES), F32),
        pltpu.VMEM((8, dm + 8, LANES), F32),
        pltpu.VMEM((12, dm, LANES), F32),
        pltpu.VMEM((ngrp, GP * CP, LANES), F32),
        pltpu.VMEM((ngrp, GP * CP, LANES), F32),
        pltpu.VMEM((RING, GP, 2, T, LANES), I32),
        pltpu.VMEM((RING, 4, GP * CP, LANES), F32),
        pltpu.VMEM((RING, 4, GP * CP, LANES), F32),
        pltpu.VMEM((RING, GP, NCH, LANES), F32),
        pltpu.VMEM((RING, GP, LANES), F32),
        pltpu.VMEM((RING, GP, LANES), I32),
        pltpu.VMEM((RING, GP, T, LANES), I32),
        pltpu.VMEM((T, LANES), I32),
        pltpu.VMEM((T // 2, LANES), I32),
        pltpu.SemaphoreType.DMA((PRE,)),
        pltpu.SemaphoreType.DMA((dm // LANES,)),
        pltpu.SemaphoreType.DMA((3,)),
        pltpu.SemaphoreType.DMA((4,)),
    ]
    out = pl.pallas_call(
        functools.partial(_kernel, seq=seq, dm=dm, heads=heads, dh=dh, nmem=nmem, seg=seg),
        out_shape=jax.ShapeDtypeStruct((seq, 2 * dm), BF16),
        in_specs=[hbm] * 7 + [vmem, vmem, hbm, vmem] + [hbm] * 4,
        out_specs=hbm,
        scratch_shapes=scratch,
        compiler_params=pltpu.CompilerParams(vmem_limit_bytes=100 * 2**20),
        name="s4_rmt",
    )(A_u.reshape(seq, dm), A_A_re, A_A_im, A_B_re, A_B_im, A_C_re, A_C_im, A_log_dt, A_Dskip,
      B_x.reshape(seq, dm), B_mem0.reshape(nmem, dm),
      *(w.reshape(dm // 8, 8 * heads, dh) for w in (B_Wq, B_Wk, B_Wv)),
      B_Wo.reshape(heads * dh, dm))
    return out.reshape(bsz, seq, 2 * dm)
```
